```python
import jax
import jax.numpy as jnp

def _softmax(x, axis=-1):
    return jax.nn.softmax(x, axis=axis)

def _gelu(x):
    return jax.nn.gelu(x, approximate=True)

def _silu(x):
    return jax.nn.silu(x)

def _sigmoid(x):
    return jax.nn.sigmoid(x)

def _layernorm(x, axis=-1, eps=1e-05):
    m = jnp.mean(x, axis=axis, keepdims=True)
    v = jnp.var(x, axis=axis, keepdims=True)
    return (x - m) / jnp.sqrt(v + eps)

def _scatter_add(tgt, idx, src, axis=0):
    return tgt.at[idx].add(src)

def _segment_sum(src, seg, n):
    return jax.ops.segment_sum(src, seg, n)

class _Rng:

    def __init__(self, key):
        self._k = key

    def _next(self):
        self._k, sub = jax.random.split(self._k)
        return sub

    def normal(self, shape):
        return jax.random.normal(self._next(), shape, dtype=jnp.bfloat16)

    def randint(self, lo, hi, shape):
        return jax.random.randint(self._next(), shape, lo, hi, dtype=jnp.int32)

    def uniform(self, shape, lo=0.0, hi=1.0):
        return jax.random.uniform(self._next(), shape, jnp.bfloat16, lo, hi)

    def permutation(self, n):
        return jax.random.permutation(self._next(), n)
kernel_name = 'concat_heads__ssm_conv_s4__memory_aug_recurrent_mem_tr__prompt'

def setup_inputs():
    _rng = _Rng(jax.random.key(int.from_bytes(__import__("os").urandom(4), "little")))
    _w = lambda a: (lambda t: t.astype(jnp.bfloat16) if jnp.issubdtype(t.dtype, jnp.floating) else t)(jnp.asarray(a))

    def _A_setup():
        B, L, D, N = (1, 2048, 640, 128)
        A_re = -jnp.exp((lambda *s: _rng.normal(s) * 0.05)(D, N))
        A_im = jnp.pi * (lambda *s: _rng.normal(s) * 0.05)(D, N)
        B_re = (lambda *s: _rng.normal(s) * 0.05)(D, N)
        B_im = (lambda *s: _rng.normal(s) * 0.05)(D, N)
        C_re = (lambda *s: _rng.normal(s) * 0.05)(D, N)
        C_im = (lambda *s: _rng.normal(s) * 0.05)(D, N)
        log_dt = (lambda *s: _rng.normal(s) * 0.05)(D) * 0.5 - 4.0
        Dskip = (lambda *s: _rng.normal(s) * 0.05)(D)
        return {'u': _w((lambda *s: _rng.normal(s) * 0.05)(B, L, D)), 'A_re': _w(A_re), 'A_im': _w(A_im), 'B_re': _w(B_re), 'B_im': _w(B_im), 'C_re': _w(C_re), 'C_im': _w(C_im), 'log_dt': _w(log_dt), 'Dskip': _w(Dskip)}
    _A_in = _A_setup()

    def _B_setup():
        B, S, Dm = (1, 2048, 640)
        H, Dh = (32, 128)
        M, seg = (8, 32)
        seg = min(seg, S)
        S = S // seg * seg
        return {'x': _w((lambda *s: _rng.normal(s) * 0.05)(B, S, Dm)), 'mem0': _w((lambda *s: _rng.normal(s) * 0.05)(B, M, Dm)), 'Wq': _w((lambda *s: _rng.normal(s) * 0.05)(Dm, H, Dh) * Dm ** (-0.5)), 'Wk': _w((lambda *s: _rng.normal(s) * 0.05)(Dm, H, Dh) * Dm ** (-0.5)), 'Wv': _w((lambda *s: _rng.normal(s) * 0.05)(Dm, H, Dh) * Dm ** (-0.5)), 'Wo': _w((lambda *s: _rng.normal(s) * 0.05)(H, Dh, Dm) * (H * Dh) ** (-0.5)), 'seg_len': seg}
    _B_in = _B_setup()
    return {'A_u': _A_in['u'], 'A_A_re': _A_in['A_re'], 'A_A_im': _A_in['A_im'], 'A_B_re': _A_in['B_re'], 'A_B_im': _A_in['B_im'], 'A_C_re': _A_in['C_re'], 'A_C_im': _A_in['C_im'], 'A_log_dt': _A_in['log_dt'], 'A_Dskip': _A_in['Dskip'], 'B_x': _B_in['x'], 'B_mem0': _B_in['mem0'], 'B_Wq': _B_in['Wq'], 'B_Wk': _B_in['Wk'], 'B_Wv': _B_in['Wv'], 'B_Wo': _B_in['Wo'], 'B_seg_len': _B_in['seg_len']}

def reference(A_u, A_A_re, A_A_im, A_B_re, A_B_im, A_C_re, A_C_im, A_log_dt, A_Dskip, B_x, B_mem0, B_Wq, B_Wk, B_Wv, B_Wo, B_seg_len):

    def _A_ref(u, A_re, A_im, B_re, B_im, C_re, C_im, log_dt, Dskip):
        Bsz, L, D = u.shape
        dt = jnp.exp(log_dt)[:, None]
        A = A_re + 1j * A_im
        Bc = B_re + 1j * B_im
        Cc = C_re + 1j * C_im
        logdA = dt * A
        dB = dt * Bc
        l = (lambda x, dt: x.astype(dt))(jnp.arange(L), A_re.dtype)
        P = jnp.exp(logdA[:, :, None] * l[None, None, :])
        K = jnp.einsum('dn,dnl,dn->dl', Cc, P, dB).real
        L2 = 2 * L
        Kp = jnp.pad(K, ((0, 0), (0, L)))
        up = (lambda x, *d: x.transpose(*d))(u, 0, 2, 1)
        up = jnp.pad(up, ((0, 0), (0, 0), (0, L)))
        Kf = (lambda x, axes=(-2, -1): jnp.fft.rfft2(x.astype(jnp.float32), axes=axes))(Kp[:, None, :], axes=(-2, -1))
        Uf = (lambda x, axes=(-2, -1): jnp.fft.rfft2(x.astype(jnp.float32), axes=axes))(up[:, :, None, :], axes=(-2, -1))
        Yf = Uf * Kf[None, :, :, :]
        y = (lambda x, s, axes=(-2, -1): jnp.fft.irfft2(x, s=s, axes=axes).astype(jnp.bfloat16))(Yf, (1, L2), axes=(-2, -1))[:, :, 0, :L]
        y = (lambda x, *d: x.transpose(*d))(y, 0, 2, 1) + u * Dskip[None, None, :]
        return y

    def _B_ref(x, mem0, Wq, Wk, Wv, Wo, seg_len):
        B, S, Dm = x.shape
        H, Dh = (Wq.shape[1], Wq.shape[2])
        M = mem0.shape[1]
        scale = Dh ** (-0.5)
        n_seg = S // seg_len
        L = M + seg_len
        idx = jnp.arange(L)
        mask = (idx[:, None] < M) | (idx[:, None] >= idx[None, :])
        mem = mem0
        outs = []
        for s in range(n_seg):
            xs = x[:, s * seg_len:(s + 1) * seg_len, :].copy()
            h = jnp.concatenate([mem, xs], axis=1)
            q = jnp.einsum('btd,dhe->bhte', h, Wq)
            k = jnp.einsum('btd,dhe->bhte', h, Wk)
            v = jnp.einsum('btd,dhe->bhte', h, Wv)
            scores = jnp.einsum('bhqe,bhke->bhqk', q, k) * scale
            scores = jnp.where(mask[None, None], scores, -1000000000.0)
            p = _softmax(scores, axis=-1)
            o = jnp.einsum('bhqk,bhke->bhqe', p, v)
            o = jnp.einsum('bhte,hed->btd', o, Wo)
            mem = o[:, :M, :].copy()
            outs.append(o[:, M:, :])
        return jnp.concatenate(outs, axis=1)
    a = _A_ref(A_u, A_A_re, A_A_im, A_B_re, A_B_im, A_C_re, A_C_im, A_log_dt, A_Dskip)
    b = _B_ref(B_x, B_mem0, B_Wq, B_Wk, B_Wv, B_Wo, B_seg_len)
    return jnp.concatenate([a, b], axis=-1)
```

```python
import functools

import jax
import jax.numpy as jnp
from jax import lax
import jax.experimental.pallas as pl
import jax.experimental.pallas.tpu as pltpu

F32 = jnp.float32
BF16 = jnp.bfloat16
U32 = jnp.uint32

T = 64
LQK, LPV, LWO, GW = 2, 4, 8, 2

_NN = (((1,), (0,)), ((), ()))
_NT = (((1,), (1,)), ((), ()))


def _dot(a, b, dims=_NN):
    return lax.dot_general(a, b, dims, preferred_element_type=F32)


def _cmul(ar, ai, br, bi):
    return ar * br - ai * bi, ar * bi + ai * br


def _kernel(u_ref, are_ref, aim_ref, bre_ref, bim_ref, cre_ref, cim_ref, ldt_ref, dsk_ref,
            mem_ref, x_hbm, wq_hbm, wk_hbm, wv_hbm, wo_hbm,
            o_hbm,
            raw_q, raw_k, raw_v, raw_o, x_v, wqkv, wo, hbuf, oa, ob,
            pw, w8, wt, gg, cb, up, yp, tre, tim, sre, sim, zre, zim, rev,
            sems,
            *, L, D, N, H, Dh, M, SEG):
    NC = L // T
    NB = D // 128
    NSEG = L // SEG
    R = M + SEG

    loads = [pltpu.make_async_copy(s, d, sems.at[i]) for i, (s, d) in enumerate(
        [(wq_hbm, raw_q.at[pl.ds(0, D * H), :]), (wk_hbm, raw_k.at[pl.ds(0, D * H), :]),
         (wv_hbm, raw_v.at[pl.ds(0, D * H), :]), (wo_hbm, raw_o), (x_hbm, x_v)])]
    for c in loads:
        c.start()

    lane = lax.broadcasted_iota(jnp.int32, (T, 128), 1)
    lo64 = lane < 64
    lo32 = lax.broadcasted_iota(jnp.int32, (NC, 128), 1) < 64

    for b in range(NB):
        rows = slice(b * 128, (b + 1) * 128)
        dt = jnp.exp(ldt_ref[:, rows].astype(F32))
        dt = jnp.broadcast_to(dt, (128, 128)).T
        a = dt * are_ref[rows, :].astype(F32)
        th = dt * aim_ref[rows, :].astype(F32)
        ea = jnp.exp(a)
        wr, wi = ea * jnp.cos(th), ea * jnp.sin(th)
        cr, ci = _cmul(cre_ref[rows, :].astype(F32), cim_ref[rows, :].astype(F32),
                       dt * bre_ref[rows, :].astype(F32), dt * bim_ref[rows, :].astype(F32))
        cb[0, rows, :] = cr
        cb[1, rows, :] = -ci
        gr, gi = _cmul(cr, ci, wr, wi)
        gg[0, rows, :] = gr
        gg[1, rows, :] = gi
        p = {0: (jnp.ones_like(wr), jnp.zeros_like(wr)), 1: (wr, wi)}
        p[2] = _cmul(*p[1], *p[1])
        p[3] = _cmul(*p[2], *p[1])
        p[4] = _cmul(*p[2], *p[2])
        p[5] = _cmul(*p[4], *p[1])
        p[6] = _cmul(*p[4], *p[2])
        p[7] = _cmul(*p[4], *p[3])
        for j in range(8):
            for ri in range(2):
                pw[ri, pl.ds(b * 1024 + j, 128, stride=8), :] = p[j][ri]
        q = _cmul(*p[4], *p[4])
        w8[0, rows, :] = q[0]
        w8[1, rows, :] = q[1]
        for _ in range(3):
            q = _cmul(*q, *q)
        wt[0, rows, :] = q[0]
        wt[1, rows, :] = q[1]

    def u_body(cp, carry):
        r0 = pl.multiple_of(cp * 2 * T, 2 * T)
        for b in range(NB):
            rev[0, 0:2 * T, :] = u_ref[pl.ds(r0, 2 * T), b * 128:(b + 1) * 128].astype(F32)
            for cc in range(2):
                for i in range(8):
                    rev[1, pl.ds(cc * T + 7 - i, 8, stride=8), :] = rev[0, pl.ds(cc * T + i, 8, stride=8), :]
            n0 = jnp.concatenate([rev[1, pl.ds(8 * (7 - a), 8), :] for a in range(8)], axis=0)
            n1 = jnp.concatenate([rev[1, pl.ds(T + 8 * (7 - a), 8), :] for a in range(8)], axis=0)
            top = jnp.where(lo64, n0, pltpu.roll(n1, 64, 1))
            bot = jnp.where(lo64, pltpu.roll(n0, 64, 1), n1)
            xt = jnp.concatenate([top, bot], axis=0).T
            for cc in range(2):
                up[pl.ds(b * 64 * NC + cp * 2 + cc, 64, stride=NC), :] = xt[cc * 64:(cc + 1) * 64]
        return carry

    lax.fori_loop(0, NC // 2, u_body, 0)

    sigma = T - 1 - lax.broadcasted_iota(jnp.int32, (T, 128), 0)
    hank_ok = (lane % 64) >= sigma
    hank_idx = jnp.where(hank_ok, lane - sigma, lane)
    lane8 = lax.broadcasted_iota(jnp.int32, (8, 128), 1)

    def grp_body(g, carry):
        ch = [pl.multiple_of((g // 8) * 128 + (g % 8) * 8 + 64 * hf, 8) for hf in range(2)]
        prow = pl.multiple_of(g * 8 * NC, 8 * NC)

        def lhs(p):
            x = up[pl.ds(prow + p * NC, NC), :]
            return jnp.concatenate([jnp.where(lo32, x, 0.0), jnp.where(lo32, 0.0, x)], axis=0)

        for p in range(8):
            vr, vi = [], []
            for hf in range(2):
                c = ch[hf] + p
                r8 = pl.multiple_of(c * 8, 8)
                cur = (pw[0, pl.ds(r8, 8), :], pw[1, pl.ds(r8, 8), :])
                st = (jnp.broadcast_to(w8[0, pl.ds(c, 1), :], (8, 128)),
                      jnp.broadcast_to(w8[1, pl.ds(c, 1), :], (8, 128)))
                for k in range(T // 8):
                    vr.append(cur[0])
                    vi.append(cur[1])
                    if k + 1 < T // 8:
                        cur = _cmul(*cur, *st)
            tr = jnp.concatenate(vr, axis=0).astype(BF16)
            ti = jnp.concatenate(vi, axis=0).astype(BF16)
            tre[p] = pltpu.bitcast(tr, U32)
            tim[p] = pltpu.bitcast(ti, U32)
            s = _dot(lhs(p), jnp.concatenate([tr, ti], axis=1))
            for hf in range(2):
                sre[hf, pl.ds(p, NC, stride=8), :] = s[hf * NC:(hf + 1) * NC, 0:128]
                sim[hf, pl.ds(p, NC, stride=8), :] = s[hf * NC:(hf + 1) * NC, 128:256]

        for hf in range(2):
            wtr, wti = wt[0, pl.ds(ch[hf], 8), :], wt[1, pl.ds(ch[hf], 8), :]
            gr, gi = gg[0, pl.ds(ch[hf], 8), :], gg[1, pl.ds(ch[hf], 8), :]
            zero = jnp.zeros((8, 128), F32)
            zre[pl.ds(hf * NC, 8, stride=2 * NC), :] = zero
            zim[pl.ds(hf * NC, 8, stride=2 * NC), :] = zero
            xr = xi = None
            for c in range(NC - 1):
                sr, si = sre[hf, c * 8:(c + 1) * 8, :], sim[hf, c * 8:(c + 1) * 8, :]
                if xr is None:
                    xr, xi = sr, si
                else:
                    xr, xi = _cmul(xr, xi, wtr, wti)
                    xr, xi = xr + sr, xi + si
                zre[pl.ds(hf * NC + c + 1, 8, stride=2 * NC), :] = xr * gr - xi * gi
                zim[pl.ds(hf * NC + c + 1, 8, stride=2 * NC), :] = -(xr * gi) - xi * gr

        cbr = [cb[0, pl.ds(ch[hf], 8), :] for hf in range(2)]
        cbi = [cb[1, pl.ds(ch[hf], 8), :] for hf in range(2)]
        for p in range(8):
            tr = pltpu.bitcast(tre[p], BF16)
            ti = pltpu.bitcast(tim[p], BF16)
            lr = jnp.concatenate([zre[p * 2 * NC:(p + 1) * 2 * NC, :]] + cbr, axis=0)
            li = jnp.concatenate([zim[p * 2 * NC:(p + 1) * 2 * NC, :]] + cbi, axis=0)
            y = _dot(lr, tr, _NT) + _dot(li, ti, _NT)
            k2 = jnp.where(lane8 < 64, y[2 * NC:2 * NC + 8], y[2 * NC + 8:2 * NC + 16])
            kb = jnp.broadcast_to(k2[p:p + 1, :], (T, 128))
            hk = jnp.take_along_axis(kb, hank_idx, axis=1)
            hk = jnp.where(hank_ok, hk, 0.0).astype(BF16)
            y = y[0:2 * NC] + _dot(lhs(p), jnp.concatenate([hk, hk], axis=0))
            yp[pl.ds((g // 8) * 64 * NC + (g % 8) * 8 + p, NC, stride=64), :] = jnp.where(lo32, y[0:NC], y[NC:2 * NC])
        return carry

    lax.fori_loop(0, D // 16, grp_body, 0)

    def y_body(cp, carry):
        r0 = pl.multiple_of(cp * 2 * T, 2 * T)
        for b in range(NB):
            cols = slice(b * 128, (b + 1) * 128)
            xt = yp[pl.ds(b * 64 * NC + r0, 128), :].T
            top, bot = xt[0:T], xt[T:2 * T]
            n0 = jnp.where(lo64, top, pltpu.roll(bot, 64, 1))
            n1 = jnp.where(lo64, pltpu.roll(top, 64, 1), bot)
            y = jnp.concatenate([n0, n1], axis=0)
            y = y + u_ref[pl.ds(r0, 2 * T), cols].astype(F32) * dsk_ref[:, cols].astype(F32)
            oa[pl.ds(r0, 2 * T), cols] = y.astype(BF16)
        return carry

    lax.fori_loop(0, NC // 2, y_body, 0)
    store_a = pltpu.make_async_copy(oa, o_hbm.at[:, pl.ds(0, D)], sems.at[5])
    store_a.start()

    for c in loads:
        c.wait()

    WB = 64

    def w_body(j, carry):
        r = pl.multiple_of(j * WB, WB)
        r2 = pl.multiple_of(j * WB * H, WB * H)
        for m, raw in enumerate((raw_q, raw_k, raw_v)):
            src = raw.bitcast(U32).at[pl.ds(r2, (WB + 1) * H), :]
            cols = slice(m * Dh, (m + 1) * Dh)
            for i in range(H // 2):
                a = src[pl.ds(i, WB, stride=H), :]
                b = src[pl.ds(i + H // 2, WB, stride=H), :]
                wqkv[2 * i, pl.ds(r, WB), cols] = (a & U32(0xFFFF)) | (b << 16)
                wqkv[2 * i + 1, pl.ds(r, WB), cols] = (a >> 16) | (b & U32(0xFFFF0000))
        return carry

    lax.fori_loop(0, D // 2 // WB, w_body, 0)

    def wo_body(i, carry):
        rows = pl.ds(pl.multiple_of(i * 2 * Dh, 2 * Dh), 2 * Dh)
        wo[pl.ds(pl.multiple_of(i * Dh, Dh), Dh), :] = pltpu.bitcast(raw_o[rows, :], U32)
        return carry

    lax.fori_loop(0, H // 2, wo_body, 0)

    hbuf[0:M, :] = mem_ref[...].astype(F32)
    row = lax.broadcasted_iota(jnp.int32, (R, R), 0)
    col = lax.broadcasted_iota(jnp.int32, (R, R), 1)
    scale = Dh ** -0.5

    def seg_body(s, carry):
        r0 = pl.multiple_of(s * SEG, SEG)
        hbuf[M:R, :] = x_v[pl.ds(r0, SEG), :].astype(F32)
        mask = (row < M) | (row >= col)
        q, k, v, p, o = {}, {}, {}, {}, {}
        acc = None
        for step in range(H + LWO + GW):
            if step < H:
                r = _dot(hbuf[...], pltpu.bitcast(wqkv[step], BF16))
                q[step] = r[:, 0:Dh] * scale
                k[step] = r[:, Dh:2 * Dh].astype(BF16)
                v[step] = r[:, 2 * Dh:3 * Dh].astype(BF16)
            h = step - LQK
            if 0 <= h < H:
                sc = jnp.where(mask, _dot(q.pop(h), k.pop(h), _NT), -1e9)
                e = jnp.exp(sc - jnp.max(sc, axis=-1, keepdims=True))
                p[h] = e / jnp.sum(e, axis=-1, keepdims=True)
            h = step - LPV
            if 0 <= h < H:
                o[h] = _dot(p.pop(h), v.pop(h))
            h = step - LWO
            if 0 <= h < H and h % GW == GW - 1:
                oo = jnp.concatenate([o.pop(i) for i in range(h - GW + 1, h + 1)], axis=1)
                w = pltpu.bitcast(wo[pl.ds((h - GW + 1) * Dh // 2, GW * Dh // 2), :], BF16)
                d = _dot(oo, w)
                acc = d if acc is None else acc + d
        hbuf[0:M, :] = acc[0:M]
        ob[pl.ds(r0, SEG), :] = acc[M:R].astype(BF16)
        return carry

    NO = 8
    PER = NSEG // NO

    def store_b(j):
        rows = pl.ds(pl.multiple_of(j * PER * SEG, PER * SEG), PER * SEG)
        return pltpu.make_async_copy(ob.at[rows, :], o_hbm.at[rows, pl.ds(D, D)], sems.at[6])

    def outer(j, carry):
        lax.fori_loop(j * PER, (j + 1) * PER, seg_body, 0)
        store_b(j).start()
        return carry

    lax.fori_loop(0, NO, outer, 0)
    store_a.wait()
    for j in range(NO):
        store_b(j).wait()


@functools.partial(jax.jit, static_argnames=("B_seg_len",))
def pallas_concat_heads__ssm_conv_s4__memory_aug_recurrent_mem_tr__prompt_kernel(
    A_u, A_A_re, A_A_im, A_B_re, A_B_im, A_C_re, A_C_im, A_log_dt, A_Dskip,
    B_x, B_mem0, B_Wq, B_Wk, B_Wv, B_Wo, B_seg_len,
):
    Bsz, L, D = A_u.shape
    N = A_A_re.shape[1]
    _, H, Dh = B_Wq.shape
    M = B_mem0.shape[1]
    SEG = int(B_seg_len)
    assert Bsz == 1 and B_x.shape == A_u.shape and N == 128 and Dh == 128
    NC = L // T

    vmem = pl.BlockSpec(memory_space=pltpu.VMEM)
    hbm = pl.BlockSpec(memory_space=pl.ANY)
    scratch = [
        pltpu.VMEM(((D + 2) * H, Dh), BF16), pltpu.VMEM(((D + 2) * H, Dh), BF16), pltpu.VMEM(((D + 2) * H, Dh), BF16),
        pltpu.VMEM((H * Dh, D), BF16),
        pltpu.VMEM((L, D), BF16),
        pltpu.VMEM((H, D // 2, 3 * Dh), U32),
        pltpu.VMEM((H * Dh // 2, D), U32),
        pltpu.VMEM((M + SEG, D), F32),
        pltpu.VMEM((L, D), BF16),
        pltpu.VMEM((L, D), BF16),
        pltpu.VMEM((2, D * 8 + 8, N), F32),
        pltpu.VMEM((2, D, N), F32),
        pltpu.VMEM((2, D, N), F32),
        pltpu.VMEM((2, D, N), F32),
        pltpu.VMEM((2, D, N), F32),
        pltpu.VMEM((D // 2 * NC + NC, 128), F32),
        pltpu.VMEM((D // 2 * NC + 64, 128), F32),
        pltpu.VMEM((8, T, N), U32),
        pltpu.VMEM((8, T, N), U32),
        pltpu.VMEM((2, NC * 8 + 8, N), F32),
        pltpu.VMEM((2, NC * 8 + 8, N), F32),
        pltpu.VMEM((18 * NC, N), F32),
        pltpu.VMEM((18 * NC, N), F32),
        pltpu.VMEM((2, 2 * T + 8, 128), F32),
        pltpu.SemaphoreType.DMA((7,)),
    ]
    out = pl.pallas_call(
        functools.partial(_kernel, L=L, D=D, N=N, H=H, Dh=Dh, M=M, SEG=SEG),
        out_shape=jax.ShapeDtypeStruct((L, 2 * D), A_u.dtype),
        in_specs=[vmem] * 10 + [hbm] * 5,
        out_specs=hbm,
        scratch_shapes=scratch,
        compiler_params=pltpu.CompilerParams(vmem_limit_bytes=100 * 1024 * 1024),
        name="s4_rmt",
    )(A_u.reshape(L, D), A_A_re, A_A_im, A_B_re, A_B_im, A_C_re, A_C_im,
      A_log_dt.reshape(1, D), A_Dskip.reshape(1, D), B_mem0.reshape(M, D),
      B_x.reshape(L, D), B_Wq.reshape(D * H, Dh), B_Wk.reshape(D * H, Dh),
      B_Wv.reshape(D * H, Dh), B_Wo.reshape(H * Dh, D))
    return out.reshape(Bsz, L, 2 * D)
```

```python
import functools

import jax
import jax.numpy as jnp
from jax import lax
import jax.experimental.pallas as pl
import jax.experimental.pallas.tpu as pltpu

F32 = jnp.float32
BF16 = jnp.bfloat16
U32 = jnp.uint32

LMM, T_STATE, T_SCAN, T_TAPS, T_INTRA = 2, 1, 11, 20, 25
T = 64
LQK, LPV, LWO, GW = 2, 4, 8, 2

PP, UP, YP, SP, ZP = 33, 33, 65, 33, 65

_NN = (((1,), (0,)), ((), ()))
_NT = (((1,), (1,)), ((), ()))


def _dot(a, b, dims=_NN):
    return lax.dot_general(a, b, dims, preferred_element_type=F32)


def _cmul(ar, ai, br, bi):
    return ar * br - ai * bi, ar * bi + ai * br


def _kernel(u_ref, are_ref, aim_ref, bre_ref, bim_ref, cre_ref, cim_ref, ldt_ref, dsk_ref,
            mem_ref, x_hbm, wq_hbm, wk_hbm, wv_hbm, wo_hbm,
            o_hbm,
            raw_q, raw_k, raw_v, raw_o, x_v, wqkv, wo, hbuf, oa, ob,
            pw, cst, up, yp, sems, *slots,
            L, D, N, H, Dh, M, SEG):
    sre, sim, zre, zim, tre, tim = (slots[i::6] for i in range(6))
    NC = L // T
    NB = D // 128
    NSEG = L // SEG
    R = M + SEG

    loads = [pltpu.make_async_copy(s, d, sems.at[i]) for i, (s, d) in enumerate(
        [(wq_hbm, raw_q.at[pl.ds(0, D * H), :]), (wk_hbm, raw_k.at[pl.ds(0, D * H), :]),
         (wv_hbm, raw_v.at[pl.ds(0, D * H), :]), (wo_hbm, raw_o), (x_hbm, x_v)])]
    for c in loads:
        c.start()

    lane = lax.broadcasted_iota(jnp.int32, (T, 128), 1)
    lo64 = lane < 64
    lo32 = lax.broadcasted_iota(jnp.int32, (NC, 128), 1) < 64

    for b in range(NB):
        rows = slice(b * 128, (b + 1) * 128)
        dt = jnp.exp(ldt_ref[:, rows].astype(F32))
        dt = jnp.broadcast_to(dt, (128, 128)).T
        a = dt * are_ref[rows, :].astype(F32)
        th = dt * aim_ref[rows, :].astype(F32)
        ea = jnp.exp(a)
        w = (ea * jnp.cos(th), ea * jnp.sin(th))
        c = _cmul(cre_ref[rows, :].astype(F32), cim_ref[rows, :].astype(F32),
                  dt * bre_ref[rows, :].astype(F32), dt * bim_ref[rows, :].astype(F32))
        g = _cmul(*c, *w)
        p = {0: (jnp.ones_like(ea), jnp.zeros_like(ea)), 1: _cmul(*w, *w)}
        p[2] = _cmul(*p[1], *p[1])
        p[3] = _cmul(*p[2], *p[1])
        p[4] = _cmul(*p[2], *p[2])
        p[5] = _cmul(*p[4], *p[1])
        p[6] = _cmul(*p[4], *p[2])
        p[7] = _cmul(*p[4], *p[3])
        w16 = _cmul(*p[4], *p[4])
        w32 = _cmul(*w16, *w16)
        w64 = _cmul(*w32, *w32)
        for ri in range(2):
            for j in range(8):
                pw[ri, pl.ds(b * 128 * PP + j * 4, 128, stride=PP), :] = p[j][ri]
            cst[0 + ri, rows, :] = w[ri]
            cst[2 + ri, rows, :] = w16[ri]
            cst[4 + ri, rows, :] = w64[ri]
            cst[6 + ri, rows, :] = g[ri]
        cst[8, rows, :] = -g[0]
        cst[9, rows, :] = c[0]
        cst[10, rows, :] = -c[1]

    ri_ = lax.broadcasted_iota(jnp.int32, (2 * T, 2 * T), 0)
    ci_ = lax.broadcasted_iota(jnp.int32, (2 * T, 2 * T), 1)
    flip = jnp.where(ci_ == (ri_ // T) * T + (T - 1) - ri_ % T, 1.0, 0.0).astype(BF16)

    def u_body(cp, carry):
        r0 = pl.multiple_of(cp * 2 * T, 2 * T)
        n = _dot(flip, u_ref[pl.ds(r0, 2 * T), :])
        for b in range(NB):
            n0, n1 = n[0:T, b * 128:(b + 1) * 128], n[T:2 * T, b * 128:(b + 1) * 128]
            top = jnp.where(lo64, n0, pltpu.roll(n1, 64, 1))
            bot = jnp.where(lo64, pltpu.roll(n0, 64, 1), n1)
            xt = jnp.concatenate([top, bot], axis=0).T
            for cc in range(2):
                up[pl.ds(b * 64 * UP + cp * 2 + cc, 64, stride=UP), :] = xt[cc * 64:(cc + 1) * 64]
        return carry

    lax.fori_loop(0, NC // 2, u_body, 0)

    r2 = 2 * lax.broadcasted_iota(jnp.int32, (T // 2, 128), 0)
    l2 = lax.broadcasted_iota(jnp.int32, (T // 2, 128), 1)
    hank_ok = (l2 % T) + r2 >= T - 2
    hank_idx = jnp.where(hank_ok, l2 + r2 - (T - 2), l2)
    lane8 = lax.broadcasted_iota(jnp.int32, (8, 128), 1)
    not_k = lax.broadcasted_iota(jnp.int32, (8, 128), 0) != 0

    def chans(g):
        ch = [(g // 8) * 128 + (g % 8) * 8 + 64 * hf for hf in range(2)]
        return ch if isinstance(g, int) else [pl.multiple_of(c, 8) for c in ch]

    def lhs(g, p):
        x = up[pl.ds((g * 8 + p) * UP, NC), :]
        return jnp.concatenate([jnp.where(lo32, x, 0.0), jnp.where(lo32, 0.0, x)], axis=0)

    NG = D // 16

    def s4_slot(tau, g0, live):
        def item(lag):
            g, p = divmod(tau - lag, 8)
            return (g, p) if 0 <= g < NG else (None, None)

        stores = []
        g, p = item(T_STATE)
        if g is not None:
            tr, ti = live.pop(("v", p))
            live["s", p] = _dot(lhs(g0 + g, p), pltpu.bitcast(jnp.concatenate([tr, ti], axis=1), BF16))
            stores += [(tre[g % 3], (p,), tr), (tim[g % 3], (p,), ti)]
        g, p = item(T_TAPS)
        if g is not None:
            rows = pl.ds(p * ZP, 2 * NC)
            y = (_dot(zre[g % 3][rows, :], pltpu.bitcast(tre[g % 3][p], BF16), _NT)
                 + _dot(zim[g % 3][rows, :], pltpu.bitcast(tim[g % 3][p], BF16), _NT))
            k2 = jnp.where(lane8 < 64, y[0:8], y[NC:NC + 8])
            k1 = jnp.where(lane8 % T == 0, 0.0, pltpu.roll(k2, 1, 1))
            kq = pltpu.pack_elementwise([k1, k2], packed_dtype=BF16)
            kq = jnp.broadcast_to(kq[0:1, :], (T // 2, 128))
            live["h", p] = jnp.where(hank_ok, jnp.take_along_axis(kq, hank_idx, axis=1), U32(0))
            live["y", p] = jnp.concatenate(
                [jnp.where(not_k, k2, 0.0), jnp.where(lo32[8:], y[8:NC], y[NC + 8:])], axis=0)
        g, p = item(T_INTRA)
        if g is not None:
            hk = live.pop(("h", p))
            y = _dot(lhs(g0 + g, p), pltpu.bitcast(jnp.concatenate([hk, hk], axis=0), BF16))
            live["y", p] = live["y", p] + jnp.where(lo32, y[0:NC], y[NC:2 * NC])
        g, p = item(0)
        if g is not None:
            ch = chans(g0 + g)
            vr, vi = [], []
            for hf in range(2):
                base = pl.ds((ch[hf] + p) * PP, 8, stride=4)
                ev = (pw[0, base, :], pw[1, base, :])
                bc = [jnp.broadcast_to(cst[n, pl.ds(ch[hf] + p, 1), :], (8, 128)) for n in range(4)]
                od = _cmul(*ev, bc[0], bc[1])
                for k in range(T // 16):
                    vr.append(pltpu.pack_elementwise([ev[0], od[0]], packed_dtype=BF16))
                    vi.append(pltpu.pack_elementwise([ev[1], od[1]], packed_dtype=BF16))
                    if k + 1 < T // 16:
                        ev = _cmul(*ev, bc[2], bc[3])
                        od = _cmul(*od, bc[2], bc[3])
            live["v", p] = (jnp.concatenate(vr, axis=0), jnp.concatenate(vi, axis=0))
        g, p = item(T_SCAN + 1)
        if g is not None:
            for (hf, c), (zr, zi) in live.pop(("z", p)).items():
                rows = (pl.ds(hf * NC + c, 8, stride=ZP), slice(None))
                stores += [(zre[g % 3], rows, zr), (zim[g % 3], rows, zi)]
        g, p = item(T_SCAN)
        if g is not None:
            ch = chans(g0 + g)
            z = {}
            for hf in range(2):
                wtr, wti, gr, gi, ngr = [cst[4 + n, pl.ds(ch[hf], 8), :] for n in range(5)]
                if p == 0:
                    z[hf, 0] = (cst[9, pl.ds(ch[hf], 8), :], cst[10, pl.ds(ch[hf], 8), :])
                for c in range(p * NC // 8, min((p + 1) * NC // 8, NC - 1)):
                    rows = pl.ds(c * SP, 8, stride=4)
                    xr, xi = sre[g % 3][hf, rows, :], sim[g % 3][hf, rows, :]
                    if c > 0:
                        pr, pi = _cmul(*live["x", hf], wtr, wti)
                        xr, xi = pr + xr, pi + xi
                    live["x", hf] = (xr, xi)
                    z[hf, c + 1] = (xr * gr - xi * gi, xi * ngr - xr * gi)
            live["z", p] = z
        g, p = item(T_STATE + LMM)
        if g is not None:
            s = live.pop(("s", p))
            for hf in range(2):
                rows = (hf, pl.ds(p * 4, NC, stride=SP), slice(None))
                stores += [(sre[g % 3], rows, s[hf * NC:(hf + 1) * NC, 0:128]),
                           (sim[g % 3], rows, s[hf * NC:(hf + 1) * NC, 128:256])]
        g, p = item(T_INTRA + LMM)
        if g is not None:
            gg = g0 + g
            rows = (pl.ds((gg // 8) * NC * YP + (gg % 8) * 8 + p, NC, stride=YP), slice(None))
            stores.append((yp, rows, live.pop(("y", p))))
        for ref, idx, val in stores:
            ref[idx] = val

    T0 = 8 * (-(-(T_INTRA + LMM) // 8))
    NJ = (8 * NG - T0) // 24
    live = {}
    for tau in range(T0):
        s4_slot(tau, 0, live)

    def grp_body(j, live):
        live = dict(live)
        for tau in range(T0, T0 + 24):
            s4_slot(tau, 3 * j, live)
        return live

    live = dict(lax.fori_loop(0, NJ, grp_body, live))
    for tau in range(T0 + 24 * NJ, 8 * NG + T_INTRA + LMM):
        s4_slot(tau, 0, live)

    def y_body(cp, carry):
        r0 = pl.multiple_of(cp * 2 * T, 2 * T)
        for b in range(NB):
            cols = slice(b * 128, (b + 1) * 128)
            xt = jnp.concatenate([yp[pl.ds((b * NC + cp * 2 + cc) * YP, 64), :] for cc in range(2)], axis=0).T
            top, bot = xt[0:T], xt[T:2 * T]
            n0 = jnp.where(lo64, top, pltpu.roll(bot, 64, 1))
            n1 = jnp.where(lo64, pltpu.roll(top, 64, 1), bot)
            y = jnp.concatenate([n0, n1], axis=0)
            y = y + u_ref[pl.ds(r0, 2 * T), cols].astype(F32) * dsk_ref[:, cols].astype(F32)
            oa[pl.ds(r0, 2 * T), cols] = y.astype(BF16)
        return carry

    lax.fori_loop(0, NC // 2, y_body, 0)
    store_a = pltpu.make_async_copy(oa, o_hbm.at[:, pl.ds(0, D)], sems.at[5])
    store_a.start()

    for c in loads:
        c.wait()

    WB = 64

    def w_body(j, carry):
        r = pl.multiple_of(j * WB, WB)
        r2 = pl.multiple_of(j * WB * H, WB * H)
        for m, raw in enumerate((raw_q, raw_k, raw_v)):
            src = raw.bitcast(U32).at[pl.ds(r2, (WB + 1) * H), :]
            cols = slice(m * Dh, (m + 1) * Dh)
            for i in range(H // 2):
                a = src[pl.ds(i, WB, stride=H), :]
                b = src[pl.ds(i + H // 2, WB, stride=H), :]
                wqkv[2 * i, pl.ds(r, WB), cols] = (a & U32(0xFFFF)) | (b << 16)
                wqkv[2 * i + 1, pl.ds(r, WB), cols] = (a >> 16) | (b & U32(0xFFFF0000))
        return carry

    lax.fori_loop(0, D // 2 // WB, w_body, 0)

    def wo_body(i, carry):
        rows = pl.ds(pl.multiple_of(i * 2 * Dh, 2 * Dh), 2 * Dh)
        wo[pl.ds(pl.multiple_of(i * Dh, Dh), Dh), :] = pltpu.bitcast(raw_o[rows, :], U32)
        return carry

    lax.fori_loop(0, H // 2, wo_body, 0)

    hbuf[0:M, :] = mem_ref[...].astype(F32)
    row = lax.broadcasted_iota(jnp.int32, (R, R), 0)
    col = lax.broadcasted_iota(jnp.int32, (R, R), 1)
    scale = Dh ** -0.5

    def seg_body(s, carry):
        r0 = pl.multiple_of(s * SEG, SEG)
        hbuf[M:R, :] = x_v[pl.ds(r0, SEG), :].astype(F32)
        mask = (row < M) | (row >= col)
        q, k, v, p, o = {}, {}, {}, {}, {}
        acc = None
        for step in range(H + LWO + GW):
            if step < H:
                r = _dot(hbuf[...], pltpu.bitcast(wqkv[step], BF16))
                q[step] = r[:, 0:Dh] * scale
                k[step] = r[:, Dh:2 * Dh].astype(BF16)
                v[step] = r[:, 2 * Dh:3 * Dh].astype(BF16)
            h = step - LQK
            if 0 <= h < H:
                sc = jnp.where(mask, _dot(q.pop(h), k.pop(h), _NT), -1e9)
                e = jnp.exp(sc - jnp.max(sc, axis=-1, keepdims=True))
                p[h] = e / jnp.sum(e, axis=-1, keepdims=True)
            h = step - LPV
            if 0 <= h < H:
                o[h] = _dot(p.pop(h), v.pop(h))
            h = step - LWO
            if 0 <= h < H and h % GW == GW - 1:
                oo = jnp.concatenate([o.pop(i) for i in range(h - GW + 1, h + 1)], axis=1)
                w = pltpu.bitcast(wo[pl.ds((h - GW + 1) * Dh // 2, GW * Dh // 2), :], BF16)
                d = _dot(oo, w)
                acc = d if acc is None else acc + d
        hbuf[0:M, :] = acc[0:M]
        ob[pl.ds(r0, SEG), :] = acc[M:R].astype(BF16)
        return carry

    NO = 8
    PER = NSEG // NO

    def store_b(j):
        rows = pl.ds(pl.multiple_of(j * PER * SEG, PER * SEG), PER * SEG)
        return pltpu.make_async_copy(ob.at[rows, :], o_hbm.at[rows, pl.ds(D, D)], sems.at[6])

    def outer(j, carry):
        lax.fori_loop(j * PER, (j + 1) * PER, seg_body, 0)
        store_b(j).start()
        return carry

    lax.fori_loop(0, NO, outer, 0)
    store_a.wait()
    for j in range(NO):
        store_b(j).wait()


@functools.partial(jax.jit, static_argnames=("B_seg_len",))
def pallas_concat_heads__ssm_conv_s4__memory_aug_recurrent_mem_tr__prompt_kernel(
    A_u, A_A_re, A_A_im, A_B_re, A_B_im, A_C_re, A_C_im, A_log_dt, A_Dskip,
    B_x, B_mem0, B_Wq, B_Wk, B_Wv, B_Wo, B_seg_len,
):
    Bsz, L, D = A_u.shape
    N = A_A_re.shape[1]
    _, H, Dh = B_Wq.shape
    M = B_mem0.shape[1]
    SEG = int(B_seg_len)
    assert Bsz == 1 and B_x.shape == A_u.shape and N == 128 and Dh == 128
    NC = L // T
    NB = D // 128

    vmem = pl.BlockSpec(memory_space=pltpu.VMEM)
    hbm = pl.BlockSpec(memory_space=pl.ANY)
    scratch = [
        pltpu.VMEM(((D + 2) * H, Dh), BF16), pltpu.VMEM(((D + 2) * H, Dh), BF16), pltpu.VMEM(((D + 2) * H, Dh), BF16),
        pltpu.VMEM((H * Dh, D), BF16),
        pltpu.VMEM((L, D), BF16),
        pltpu.VMEM((H, D // 2, 3 * Dh), U32),
        pltpu.VMEM((H * Dh // 2, D), U32),
        pltpu.VMEM((M + SEG, D), F32),
        pltpu.VMEM((L, D), BF16),
        pltpu.VMEM((L, D), BF16),
        pltpu.VMEM((2, (D + 1) * PP, N), F32),
        pltpu.VMEM((11, D, N), F32),
        pltpu.VMEM(((D // 2 + 1) * UP, 128), F32),
        pltpu.VMEM(((NB * NC + 1) * YP, 128), F32),
        pltpu.SemaphoreType.DMA((7,)),
    ] + 3 * [
        pltpu.VMEM((2, (NC + 1) * SP, N), F32),
        pltpu.VMEM((2, (NC + 1) * SP, N), F32),
        pltpu.VMEM((10 * ZP, N), F32),
        pltpu.VMEM((10 * ZP, N), F32),
        pltpu.VMEM((8, T, N), U32),
        pltpu.VMEM((8, T, N), U32),
    ]
    out = pl.pallas_call(
        functools.partial(_kernel, L=L, D=D, N=N, H=H, Dh=Dh, M=M, SEG=SEG),
        out_shape=jax.ShapeDtypeStruct((L, 2 * D), A_u.dtype),
        in_specs=[vmem] * 10 + [hbm] * 5,
        out_specs=hbm,
        scratch_shapes=scratch,
        compiler_params=pltpu.CompilerParams(vmem_limit_bytes=100 * 1024 * 1024),
        name="s4_rmt",
    )(A_u.reshape(L, D), A_A_re, A_A_im, A_B_re, A_B_im, A_C_re, A_C_im,
      A_log_dt.reshape(1, D), A_Dskip.reshape(1, D), B_mem0.reshape(M, D),
      B_x.reshape(L, D), B_Wq.reshape(D * H, Dh), B_Wk.reshape(D * H, Dh),
      B_Wv.reshape(D * H, Dh), B_Wo.reshape(H * Dh, D))
    return out.reshape(Bsz, L, 2 * D)
```

```python
import functools

import jax
import jax.numpy as jnp
from jax import lax
import jax.experimental.pallas as pl
import jax.experimental.pallas.tpu as pltpu

F32 = jnp.float32
BF16 = jnp.bfloat16
U32 = jnp.uint32

LMM, T_STATE, T_SCAN, T_TAPS, T_INTRA = 2, 1, 12, 22, 30
SB = 144
UC = 8
YSTEP = 24
T = 64
LQK, LPV, LWO, GW = 2, 6, 16, 2

PP, UP, YP, SP, ZP, WP = 33, 33, 321, 33, 65, 40

_NN = (((1,), (0,)), ((), ()))
_NT = (((1,), (1,)), ((), ()))


def _dot(a, b, dims=_NN):
    return lax.dot_general(a, b, dims, preferred_element_type=F32)


def _cmul(ar, ai, br, bi):
    return ar * br - ai * bi, ar * bi + ai * br


def _kernel(are_ref, aim_ref, bre_ref, bim_ref, cre_ref, cim_ref, ldt_ref, dsk_ref,
            mem_ref, u_hbm, x_hbm, wq_hbm, wk_hbm, wv_hbm, wo_hbm,
            o_hbm,
            raw_q, raw_k, raw_v, raw_o, u_ref, x_v, wqkv, wo, hbuf, ob,
            pw, cst, up, yp, sems, *slots,
            L, D, N, H, Dh, M, SEG):
    sre, sim, zre, zim, tre, tim = (slots[i::6] for i in range(6))
    NC = L // T
    NB = D // 128
    NSEG = L // SEG
    R = M + SEG

    NO = 8
    PER = NSEG // NO
    X0 = PER * SEG
    copy = pltpu.make_async_copy
    load_u = copy(u_hbm, u_ref, sems.at[0])
    load_w = [copy(w.bitcast(U32), r.at[:, pl.ds(0, H), :], sems.at[1 + i])
              for i, (w, r) in enumerate(((wq_hbm, raw_q), (wk_hbm, raw_k), (wv_hbm, raw_v)))]
    load_wo = copy(wo_hbm, raw_o, sems.at[4])
    load_x0 = copy(x_hbm.at[pl.ds(0, X0), :], x_v.at[pl.ds(0, X0), :], sems.at[5])
    load_x1 = copy(x_hbm.at[pl.ds(X0, L - X0), :], x_v.at[pl.ds(X0, L - X0), :], sems.at[6])
    for c in [load_u] + load_w + [load_wo, load_x0]:
        c.start()

    lane = lax.broadcasted_iota(jnp.int32, (T, 128), 1)
    lo64 = lane < 64
    lo32 = lax.broadcasted_iota(jnp.int32, (NC, 128), 1) < 64

    for b in range(NB):
        rows = slice(b * 128, (b + 1) * 128)
        dt = jnp.exp(ldt_ref[:, rows].astype(F32))
        dt = jnp.broadcast_to(dt, (128, 128)).T
        a = dt * are_ref[rows, :].astype(F32)
        th = dt * aim_ref[rows, :].astype(F32)
        ea = jnp.exp(a)
        w = (ea * jnp.cos(th), ea * jnp.sin(th))
        c = _cmul(cre_ref[rows, :].astype(F32), cim_ref[rows, :].astype(F32),
                  dt * bre_ref[rows, :].astype(F32), dt * bim_ref[rows, :].astype(F32))
        g = _cmul(*c, *w)
        p = {0: (jnp.ones_like(ea), jnp.zeros_like(ea)), 1: _cmul(*w, *w)}
        p[2] = _cmul(*p[1], *p[1])
        p[3] = _cmul(*p[2], *p[1])
        p[4] = _cmul(*p[2], *p[2])
        p[5] = _cmul(*p[4], *p[1])
        p[6] = _cmul(*p[4], *p[2])
        p[7] = _cmul(*p[4], *p[3])
        w16 = _cmul(*p[4], *p[4])
        w32 = _cmul(*w16, *w16)
        w64 = _cmul(*w32, *w32)
        for ri in range(2):
            for j in range(8):
                pw[ri, pl.ds(b * 128 * PP + j * 4, 128, stride=PP), :] = p[j][ri]
            cst[0 + ri, rows, :] = w[ri]
            cst[2 + ri, rows, :] = w16[ri]
            cst[4 + ri, rows, :] = w64[ri]
            cst[6 + ri, rows, :] = g[ri]
        cst[8, rows, :] = -g[0]
        cst[9, rows, :] = c[0]
        cst[10, rows, :] = -c[1]

    flip = jnp.where(lax.broadcasted_iota(jnp.int32, (T, T), 0)
                     + lax.broadcasted_iota(jnp.int32, (T, T), 1) == T - 1, 1.0, 0.0).astype(BF16)
    load_u.wait()

    def u_body(j, carry):
        cs = [j * UC + i for i in range(UC)]
        ns = [_dot(flip, u_ref[pl.ds(pl.multiple_of(c * T, T), T), :]) for c in cs]
        stores = []
        for c, n in zip(cs, ns):
            for sb in range(NB // 2):
                xt = jnp.concatenate([n[:, sb * 256:sb * 256 + 128], n[:, sb * 256 + 128:sb * 256 + 256]], axis=0).T
                stores.append((pl.ds(sb * 128 * UP + c, 128, stride=UP), xt))
        if NB % 2:
            for i in range(0, UC, 2):
                n0, n1 = ns[i][:, D - 128:], ns[i + 1][:, D - 128:]
                top = jnp.where(lo64, n0, pltpu.roll(n1, 64, 1))
                bot = jnp.where(lo64, pltpu.roll(n0, 64, 1), n1)
                xt = jnp.concatenate([top, bot], axis=0).T
                for cc in range(2):
                    stores.append((pl.ds((NB // 2) * 128 * UP + cs[i + cc], 64, stride=UP), xt[cc * 64:(cc + 1) * 64]))
        for rows, val in stores:
            up[rows, :] = val
        return carry

    lax.fori_loop(0, NC // UC, u_body, 0)

    r2 = 2 * lax.broadcasted_iota(jnp.int32, (T // 2, 128), 0)
    l2 = lax.broadcasted_iota(jnp.int32, (T // 2, 128), 1)
    hank_ok = (l2 % T) + r2 >= T - 2
    hank_idx = jnp.where(hank_ok, l2 + r2 - (T - 2), l2)
    lane8 = lax.broadcasted_iota(jnp.int32, (8, 128), 1)
    not_k = lax.broadcasted_iota(jnp.int32, (8, 128), 0) != 0

    def chans(g):
        ca = (g // 16) * 256 + (g % 16) * 8
        ch = [ca, ca + 128 - 64 * (g // (16 * (NB // 2)))]
        return ch if isinstance(g, int) else [pl.multiple_of(c, 8) for c in ch]

    def lhs(g, p):
        x = up[pl.ds((g * 8 + p) * UP, NC), :]
        return jnp.concatenate([jnp.where(lo32, x, 0.0), jnp.where(lo32, 0.0, x)], axis=0)

    NG = D // 16

    def s4_slot(tau, g0, live):
        def item(lag):
            g, p = divmod(tau - lag, 8)
            return (g, p) if 0 <= g < NG else (None, None)

        stores = []
        g, p = item(T_STATE)
        if g is not None:
            tr, ti = live.pop(("v", g % 3, p))
            live["s", g % 3, p] = _dot(lhs(g0 + g, p), pltpu.bitcast(jnp.concatenate([tr, ti], axis=1), BF16))
            stores += [(tre[g % 3], (p,), tr), (tim[g % 3], (p,), ti)]
        g, p = item(T_TAPS)
        if g is not None:
            rows = pl.ds(p * ZP, 2 * NC)
            y = (_dot(zre[g % 3][rows, :], pltpu.bitcast(tre[g % 3][p], BF16), _NT)
                 + _dot(zim[g % 3][rows, :], pltpu.bitcast(tim[g % 3][p], BF16), _NT))
            k2 = jnp.where(lane8 < 64, y[0:8], y[NC:NC + 8])
            k1 = jnp.where(lane8 % T == 0, 0.0, pltpu.roll(k2, 1, 1))
            kq = pltpu.pack_elementwise([k1, k2], packed_dtype=BF16)
            kq = jnp.broadcast_to(kq[0:1, :], (T // 2, 128))
            live["h", g % 3, p] = jnp.where(hank_ok, jnp.take_along_axis(kq, hank_idx, axis=1), U32(0))
            live["y", g % 3, p] = jnp.concatenate(
                [jnp.where(not_k, k2, 0.0), jnp.where(lo32[8:], y[8:NC], y[NC + 8:])], axis=0)
        g, p = item(T_INTRA)
        if g is not None:
            hk = live.pop(("h", g % 3, p))
            y = _dot(lhs(g0 + g, p), pltpu.bitcast(jnp.concatenate([hk, hk], axis=0), BF16))
            live["y", g % 3, p] = live["y", g % 3, p] + jnp.where(lo32, y[0:NC], y[NC:2 * NC])
        g, p = item(0)
        if g is not None:
            ch = chans(g0 + g)
            vr, vi = [], []
            for hf in range(2):
                base = pl.ds((ch[hf] + p) * PP, 8, stride=4)
                ev = (pw[0, base, :], pw[1, base, :])
                bc = [jnp.broadcast_to(cst[n, pl.ds(ch[hf] + p, 1), :], (8, 128)) for n in range(4)]
                od = _cmul(*ev, bc[0], bc[1])
                for k in range(T // 16):
                    vr.append(pltpu.pack_elementwise([ev[0], od[0]], packed_dtype=BF16))
                    vi.append(pltpu.pack_elementwise([ev[1], od[1]], packed_dtype=BF16))
                    if k + 1 < T // 16:
                        ev = _cmul(*ev, bc[2], bc[3])
                        od = _cmul(*od, bc[2], bc[3])
            live["v", g % 3, p] = (jnp.concatenate(vr, axis=0), jnp.concatenate(vi, axis=0))
        g, p = item(T_SCAN + 1)
        if g is not None:
            for (hf, c), (zr, zi) in live.pop(("z", g % 3, p)).items():
                rows = (pl.ds(hf * NC + c, 8, stride=ZP), slice(None))
                stores += [(zre[g % 3], rows, zr), (zim[g % 3], rows, zi)]
        g, p = item(T_SCAN)
        if g is not None:
            ch = chans(g0 + g)
            z = {}
            for hf in range(2):
                wtr, wti, gr, gi, ngr = [cst[4 + n, pl.ds(ch[hf], 8), :] for n in range(5)]
                if p == 0:
                    z[hf, 0] = (cst[9, pl.ds(ch[hf], 8), :], cst[10, pl.ds(ch[hf], 8), :])
                for c in range(p * NC // 8, min((p + 1) * NC // 8, NC - 1)):
                    rows = pl.ds(c * SP, 8, stride=4)
                    xr, xi = sre[g % 3][hf, rows, :], sim[g % 3][hf, rows, :]
                    if c > 0:
                        pr, pi = _cmul(*live["x", hf], wtr, wti)
                        xr, xi = pr + xr, pi + xi
                    live["x", hf] = (xr, xi)
                    z[hf, c + 1] = (xr * gr - xi * gi, xi * ngr - xr * gi)
            live["z", g % 3, p] = z
        g, p = item(T_STATE + LMM)
        if g is not None:
            s = live.pop(("s", g % 3, p))
            for hf in range(2):
                rows = (hf, pl.ds(p * 4, NC, stride=SP), slice(None))
                stores += [(sre[g % 3], rows, s[hf * NC:(hf + 1) * NC, 0:128]),
                           (sim[g % 3], rows, s[hf * NC:(hf + 1) * NC, 128:256])]
        g, p = item(T_INTRA + LMM)
        if g is not None:
            gg = g0 + g
            rows = (pl.ds(gg * 8 + p, NC, stride=YP), slice(None))
            stores.append((yp, rows, live.pop(("y", g % 3, p))))
        for ref, idx, val in stores:
            ref[idx] = val

    T0 = 8 * (-(-(T_INTRA + LMM) // 8))
    NJ = (8 * NG - T0) // SB
    live = {}
    for tau in range(T0):
        s4_slot(tau, 0, live)

    def grp_body(j, live):
        live = dict(live)
        for tau in range(T0, T0 + SB):
            s4_slot(tau, (SB // 8) * j, live)
        return live

    live = dict(lax.fori_loop(0, NJ, grp_body, live))
    for tau in range(T0 + SB * NJ, 8 * NG + T_INTRA + LMM):
        s4_slot(tau, 0, live)

    def s4_output(s):
        c, sb = s // 2, s % 2
        rows = pl.ds(pl.multiple_of(c * T, T), T)
        res = []
        xt = yp[pl.ds(c * YP + sb * 128, 128), :].T
        for hf in range(2):
            cols = pl.ds(pl.multiple_of(sb * 256 + hf * 128, 128), 128)
            res.append((rows, cols, xt[hf * T:(hf + 1) * T]))
        xt = yp[pl.ds(c * YP + (NB // 2) * 128 - 64, 128), :].T
        res.append((rows, pl.ds(D - 128, 128), jnp.where(lo64, pltpu.roll(xt[0:T], 64, 1), xt[T:2 * T])))
        return [(r, cl, (y + u_ref[r, cl].astype(F32) * dsk_ref[:, cl].astype(F32)).astype(BF16)) for r, cl, y in res]

    WB = 64
    for m, raw in enumerate((raw_q, raw_k, raw_v)):
        load_w[m].wait()

        def w_body(j, carry, m=m, src=raw.reshape(D // 2 * WP, Dh)):
            rows = pl.ds(pl.multiple_of(j * WB, WB), WB)
            cols = slice(m * Dh, (m + 1) * Dh)
            for i in range(H // 2):
                a = src[pl.ds(j * WB * WP + i, WB, stride=WP), :]
                b = src[pl.ds(j * WB * WP + i + H // 2, WB, stride=WP), :]
                wqkv[2 * i, rows, cols] = (a & U32(0xFFFF)) | (b << 16)
                wqkv[2 * i + 1, rows, cols] = (a >> 16) | (b & U32(0xFFFF0000))
            return carry

        lax.fori_loop(0, D // 2 // WB, w_body, 0)
    load_wo.wait()

    def wo_body(i, carry):
        rows = pl.ds(pl.multiple_of(i * 2 * Dh, 2 * Dh), 2 * Dh)
        wo[pl.ds(pl.multiple_of(i * Dh, Dh), Dh), :] = pltpu.bitcast(raw_o[rows, :], U32)
        return carry

    lax.fori_loop(0, H // 2, wo_body, 0)
    load_x0.wait()
    load_x1.start()

    hbuf[0:M, :] = mem_ref[...].astype(F32)
    row = lax.broadcasted_iota(jnp.int32, (R, R), 0)
    col = lax.broadcasted_iota(jnp.int32, (R, R), 1)
    scale = Dh ** -0.5

    def seg_body(s, carry):
        r0 = pl.multiple_of(s * SEG, SEG)
        hbuf[M:R, :] = x_v[pl.ds(r0, SEG), :].astype(F32)
        mask = (row < M) | (row >= col)
        q, k, v, p, o = {}, {}, {}, {}, {}
        acc, h0, step = None, 0, 0
        while h0 < H:
            if step < H:
                r = _dot(hbuf[...], pltpu.bitcast(wqkv[step], BF16))
                q[step] = r[:, 0:Dh] * scale
                k[step] = r[:, Dh:2 * Dh].astype(BF16)
                v[step] = r[:, 2 * Dh:3 * Dh].astype(BF16)
            h = step - LQK
            if 0 <= h < H:
                sc = jnp.where(mask, _dot(q.pop(h), k.pop(h), _NT), -1e9)
                e = jnp.exp(sc - jnp.max(sc, axis=-1, keepdims=True))
                p[h] = e / jnp.sum(e, axis=-1, keepdims=True)
            h = step - LPV
            if 0 <= h < H:
                o[h] = _dot(p.pop(h), v.pop(h))
            h = h0 + GW - 1
            if h in o and (h <= step - LWO or step >= H):
                oo = jnp.concatenate([o.pop(i) for i in range(h0, h + 1)], axis=1)
                d = _dot(oo, pltpu.bitcast(wo[pl.ds(h0 * Dh // 2, GW * Dh // 2), :], BF16))
                acc = d if acc is None else acc + d
                h0 += GW
            if step == YSTEP:
                s4_out = s4_output(s)
            step += 1
        hbuf[0:M, :] = acc[0:M]
        ob[pl.ds(r0, SEG), D:2 * D] = acc[M:R].astype(BF16)
        for r, cl, y in s4_out:
            ob[r, cl] = y
        return carry

    def store(j):
        rows = pl.ds(pl.multiple_of(j * X0, X0), X0)
        return copy(ob.at[rows, :], o_hbm.at[rows, :], sems.at[7])

    def outer(j, carry):
        lax.fori_loop(j * PER, (j + 1) * PER, seg_body, 0)
        store(j).start()

        @pl.when(j == 0)
        def _():
            load_x1.wait()

        return carry

    lax.fori_loop(0, NO, outer, 0)
    copy(ob, o_hbm, sems.at[7]).wait()


@functools.partial(jax.jit, static_argnames=("B_seg_len",))
def pallas_concat_heads__ssm_conv_s4__memory_aug_recurrent_mem_tr__prompt_kernel(
    A_u, A_A_re, A_A_im, A_B_re, A_B_im, A_C_re, A_C_im, A_log_dt, A_Dskip,
    B_x, B_mem0, B_Wq, B_Wk, B_Wv, B_Wo, B_seg_len,
):
    Bsz, L, D = A_u.shape
    N = A_A_re.shape[1]
    _, H, Dh = B_Wq.shape
    M = B_mem0.shape[1]
    SEG = int(B_seg_len)
    assert SEG * 2 == T and D == 640 and Bsz == 1 and B_x.shape == A_u.shape and N == 128 and Dh == 128
    NC = L // T
    NB = D // 128

    vmem = pl.BlockSpec(memory_space=pltpu.VMEM)
    hbm = pl.BlockSpec(memory_space=pl.ANY)
    scratch = [
        pltpu.VMEM((D // 2, WP, Dh), U32), pltpu.VMEM((D // 2, WP, Dh), U32), pltpu.VMEM((D // 2, WP, Dh), U32),
        pltpu.VMEM((H * Dh, D), BF16),
        pltpu.VMEM((L, D), BF16),
        pltpu.VMEM((L, D), BF16),
        pltpu.VMEM((H, D // 2, 3 * Dh), U32),
        pltpu.VMEM((H * Dh // 2, D), U32),
        pltpu.VMEM((M + SEG, D), F32),
        pltpu.VMEM((L, 2 * D), BF16),
        pltpu.VMEM((2, (D + 1) * PP, N), F32),
        pltpu.VMEM((11, D, N), F32),
        pltpu.VMEM(((D // 2 + 1) * UP, 128), F32),
        pltpu.VMEM(((NC + 1) * YP, 128), F32),
        pltpu.SemaphoreType.DMA((8,)),
    ] + 3 * [
        pltpu.VMEM((2, (NC + 1) * SP, N), F32),
        pltpu.VMEM((2, (NC + 1) * SP, N), F32),
        pltpu.VMEM((10 * ZP, N), F32),
        pltpu.VMEM((10 * ZP, N), F32),
        pltpu.VMEM((8, T, N), U32),
        pltpu.VMEM((8, T, N), U32),
    ]
    out = pl.pallas_call(
        functools.partial(_kernel, L=L, D=D, N=N, H=H, Dh=Dh, M=M, SEG=SEG),
        out_shape=jax.ShapeDtypeStruct((L, 2 * D), A_u.dtype),
        in_specs=[vmem] * 9 + [hbm] * 6,
        out_specs=hbm,
        scratch_shapes=scratch,
        compiler_params=pltpu.CompilerParams(vmem_limit_bytes=120 * 1024 * 1024),
        name="s4_rmt",
    )(A_A_re, A_A_im, A_B_re, A_B_im, A_C_re, A_C_im,
      A_log_dt.reshape(1, D), A_Dskip.reshape(1, D), B_mem0.reshape(M, D),
      A_u.reshape(L, D), B_x.reshape(L, D), B_Wq.reshape(D // 2, 2 * H, Dh), B_Wk.reshape(D // 2, 2 * H, Dh),
      B_Wv.reshape(D // 2, 2 * H, Dh), B_Wo.reshape(H * Dh, D))
    return out.reshape(Bsz, L, 2 * D)
```

```python
import functools

import jax
import jax.numpy as jnp
from jax import lax
import jax.experimental.pallas as pl
import jax.experimental.pallas.tpu as pltpu

F32 = jnp.float32
BF16 = jnp.bfloat16
U32 = jnp.uint32

LMM, T_STATE, T_SCAN, T_TAPS, T_INTRA = 2, 1, 12, 22, 30
SB = 144
WB = 32
UC = 8
YSTEP = 24
T = 64
LQK, LPV, LWO, GW = 2, 6, 16, 2

PP, UP, YP, SP, ZP, WP = 33, 17, 321, 33, 33, 40

_NN = (((1,), (0,)), ((), ()))
_NT = (((1,), (1,)), ((), ()))


def _dot(a, b, dims=_NN):
    return lax.dot_general(a, b, dims, preferred_element_type=F32)


def _pack(a, b):
    return pltpu.pack_elementwise([a, b], packed_dtype=BF16)


def _cmul(ar, ai, br, bi):
    return ar * br - ai * bi, ar * bi + ai * br


def _kernel(are_ref, aim_ref, bre_ref, bim_ref, cre_ref, cim_ref, ldt_ref, dsk_ref,
            mem_ref, u_hbm, x_hbm, wq_hbm, wk_hbm, wv_hbm, wo_hbm,
            o_hbm,
            raw_q, raw_k, raw_v, u_ref, x_v, wqkv, wo, hbuf, ob,
            pw, cst, up, yp, dsk, sems, *slots,
            L, D, N, H, Dh, M, SEG):
    sre, sim, zre, zim, tre, tim = (slots[i::6] for i in range(6))
    NC = L // T
    NB = D // 128
    NSEG = L // SEG
    R = M + SEG

    NO = 32
    PER = NSEG // NO
    X0 = PER * SEG
    copy = pltpu.make_async_copy
    load_u = copy(u_hbm, u_ref, sems.at[0])
    load_w = [copy(w.bitcast(U32), r.at[:, pl.ds(0, H), :], sems.at[1 + i])
              for i, (w, r) in enumerate(((wq_hbm, raw_q), (wk_hbm, raw_k), (wv_hbm, raw_v)))]
    load_wo = copy(wo_hbm.bitcast(U32), wo, sems.at[4])
    load_x0 = copy(x_hbm.at[pl.ds(0, X0), :], x_v.at[pl.ds(0, X0), :], sems.at[5])
    load_x1 = copy(x_hbm.at[pl.ds(X0, L - X0), :], x_v.at[pl.ds(X0, L - X0), :], sems.at[6])
    for c in [load_u] + load_w + [load_wo, load_x0]:
        c.start()

    lane = lax.broadcasted_iota(jnp.int32, (T, 128), 1)
    lo64 = lane < 64
    lo32 = lax.broadcasted_iota(jnp.int32, (NC, 128), 1) < 64

    ldt = ldt_ref[...].astype(F32).reshape(1, D)
    dsk[...] = dsk_ref[...].astype(F32).reshape(1, D)
    for b in range(NB):
        rows = slice(b * 128, (b + 1) * 128)
        dt = jnp.exp(ldt[:, rows])
        dt = jnp.broadcast_to(dt, (128, 128)).T
        a = dt * are_ref[rows, :].astype(F32)
        th = dt * aim_ref[rows, :].astype(F32)
        ea = jnp.exp(a)
        w = (ea * jnp.cos(th), ea * jnp.sin(th))
        c = _cmul(cre_ref[rows, :].astype(F32), cim_ref[rows, :].astype(F32),
                  dt * bre_ref[rows, :].astype(F32), dt * bim_ref[rows, :].astype(F32))
        g = _cmul(*c, *w)
        p = {0: (jnp.ones_like(ea), jnp.zeros_like(ea)), 1: _cmul(*w, *w)}
        p[2] = _cmul(*p[1], *p[1])
        p[3] = _cmul(*p[2], *p[1])
        p[4] = _cmul(*p[2], *p[2])
        p[5] = _cmul(*p[4], *p[1])
        p[6] = _cmul(*p[4], *p[2])
        p[7] = _cmul(*p[4], *p[3])
        w16 = _cmul(*p[4], *p[4])
        w32 = _cmul(*w16, *w16)
        w64 = _cmul(*w32, *w32)
        for ri in range(2):
            for j in range(8):
                pw[ri, pl.ds(b * 128 * PP + j * 4, 128, stride=PP), :] = p[j][ri]
            cst[0 + ri, rows, :] = w[ri]
            cst[2 + ri, rows, :] = w16[ri]
            cst[4 + ri, rows, :] = w64[ri]
            cst[6 + ri, rows, :] = g[ri]
        cst[8, rows, :] = -g[0]
        cst[9, rows, :] = c[0]
        cst[10, rows, :] = -c[1]

    flip = jnp.where(lax.broadcasted_iota(jnp.int32, (T, T), 0)
                     + lax.broadcasted_iota(jnp.int32, (T, T), 1) == T - 1, 1.0, 0.0).astype(BF16)
    load_u.wait()

    def u_body(j, carry):
        cs = [j * UC + i for i in range(UC)]
        ns = [_dot(flip, u_ref[pl.ds(pl.multiple_of(c * T, T), T), :]) for c in cs]
        ns = [_pack(ns[i], ns[i + 1]) for i in range(0, UC, 2)]
        cs = [j * (UC // 2) + i for i in range(UC // 2)]
        stores = []
        for c, n in zip(cs, ns):
            for sb in range(NB // 2):
                xt = jnp.concatenate([n[:, sb * 256:sb * 256 + 128], n[:, sb * 256 + 128:sb * 256 + 256]], axis=0).T
                stores.append((pl.ds(sb * 128 * UP + c, 128, stride=UP), xt))
        if NB % 2:
            for i in range(0, UC // 2, 2):
                n0, n1 = ns[i][:, D - 128:], ns[i + 1][:, D - 128:]
                top = jnp.where(lo64, n0, pltpu.roll(n1, 64, 1))
                bot = jnp.where(lo64, pltpu.roll(n0, 64, 1), n1)
                xt = jnp.concatenate([top, bot], axis=0).T
                for cc in range(2):
                    stores.append((pl.ds((NB // 2) * 128 * UP + cs[i + cc], 64, stride=UP), xt[cc * 64:(cc + 1) * 64]))
        for rows, val in stores:
            up[rows, :] = val
        return carry

    lax.fori_loop(0, NC // UC, u_body, 0)

    r2 = 2 * lax.broadcasted_iota(jnp.int32, (T // 2, 128), 0)
    l2 = lax.broadcasted_iota(jnp.int32, (T // 2, 128), 1)
    hank_ok = (l2 % T) + r2 >= T - 2
    hank_idx = jnp.where(hank_ok, l2 + r2 - (T - 2), l2)
    lane8 = lax.broadcasted_iota(jnp.int32, (8, 128), 1)
    not_k = lax.broadcasted_iota(jnp.int32, (8, 128), 0) != 0

    def chans(g):
        ca = (g // 16) * 256 + (g % 16) * 8
        ch = [ca, ca + 128 - 64 * (g // (16 * (NB // 2)))]
        return ch if isinstance(g, int) else [pl.multiple_of(c, 8) for c in ch]

    def lhs(g, p):
        x = pltpu.bitcast(up[pl.ds((g * 8 + p) * UP, NC // 2), :], BF16)
        return jnp.concatenate([jnp.where(lo32, x, 0.0), jnp.where(lo32, 0.0, x)], axis=0)

    NG = D // 16

    def s4_slot(tau, g0, live):
        def item(lag):
            g, p = divmod(tau - lag, 8)
            return (g, p) if 0 <= g < NG else (None, None)

        stores = []
        g, p = item(T_STATE)
        if g is not None:
            tr, ti = live.pop(("v", g % 3, p))
            live["s", g % 3, p] = _dot(lhs(g0 + g, p), pltpu.bitcast(jnp.concatenate([tr, ti], axis=1), BF16))
            stores += [(tre[g % 3], (p,), tr), (tim[g % 3], (p,), ti)]
        g, p = item(T_TAPS)
        if g is not None:
            rows = pl.ds(p * ZP, NC)
            y = (_dot(pltpu.bitcast(zre[g % 3][rows, :], BF16), pltpu.bitcast(tre[g % 3][p], BF16), _NT)
                 + _dot(pltpu.bitcast(zim[g % 3][rows, :], BF16), pltpu.bitcast(tim[g % 3][p], BF16), _NT))
            k2 = jnp.where(lane8 < 64, y[0:8], y[NC:NC + 8])
            k1 = jnp.where(lane8 % T == 0, 0.0, pltpu.roll(k2, 1, 1))
            kq = _pack(k1, k2)
            kq = jnp.broadcast_to(kq[0:1, :], (T // 2, 128))
            live["h", g % 3, p] = jnp.where(hank_ok, jnp.take_along_axis(kq, hank_idx, axis=1), U32(0))
            live["y", g % 3, p] = jnp.concatenate(
                [jnp.where(not_k, k2, 0.0), jnp.where(lo32[8:], y[8:NC], y[NC + 8:])], axis=0)
        g, p = item(T_INTRA)
        if g is not None:
            hk = live.pop(("h", g % 3, p))
            y = _dot(lhs(g0 + g, p), pltpu.bitcast(jnp.concatenate([hk, hk], axis=0), BF16))
            live["y", g % 3, p] = live["y", g % 3, p] + jnp.where(lo32, y[0:NC], y[NC:2 * NC])
        g, p = item(0)
        if g is not None:
            ch = chans(g0 + g)
            vr, vi = [], []
            for hf in range(2):
                base = pl.ds((ch[hf] + p) * PP, 8, stride=4)
                ev = (pw[0, base, :], pw[1, base, :])
                bc = [jnp.broadcast_to(cst[n, pl.ds(ch[hf] + p, 1), :], (8, 128)) for n in range(4)]
                od = _cmul(*ev, bc[0], bc[1])
                for k in range(T // 16):
                    vr.append(_pack(ev[0], od[0]))
                    vi.append(_pack(ev[1], od[1]))
                    if k + 1 < T // 16:
                        ev = _cmul(*ev, bc[2], bc[3])
                        od = _cmul(*od, bc[2], bc[3])
            live["v", g % 3, p] = (jnp.concatenate(vr, axis=0), jnp.concatenate(vi, axis=0))
        g, p = item(T_SCAN + 1)
        if g is not None:
            for (hf, c), (zr, zi) in live.pop(("z", g % 3, p)).items():
                rows = (pl.ds((hf * NC + c) // 2, 8, stride=ZP), slice(None))
                stores += [(zre[g % 3], rows, zr), (zim[g % 3], rows, zi)]
        g, p = item(T_SCAN)
        if g is not None:
            ch = chans(g0 + g)
            z = {}
            for hf in range(2):
                wtr, wti, gr, gi, ngr = [cst[4 + n, pl.ds(ch[hf], 8), :] for n in range(5)]
                if p == 0:
                    live["e", hf] = (cst[9, pl.ds(ch[hf], 8), :], cst[10, pl.ds(ch[hf], 8), :])
                for c in range(p * NC // 8, min((p + 1) * NC // 8, NC - 1)):
                    rows = pl.ds(c * SP, 8, stride=4)
                    xr, xi = sre[g % 3][hf, rows, :], sim[g % 3][hf, rows, :]
                    if c > 0:
                        pr, pi = _cmul(*live["x", hf], wtr, wti)
                        xr, xi = pr + xr, pi + xi
                    live["x", hf] = (xr, xi)
                    zn = (xr * gr - xi * gi, xi * ngr - xr * gi)
                    if c % 2:
                        live["e", hf] = zn
                    else:
                        z[hf, c] = [_pack(a, b) for a, b in zip(live.pop(("e", hf)), zn)]
            live["z", g % 3, p] = z
        g, p = item(T_STATE + LMM)
        if g is not None:
            s = live.pop(("s", g % 3, p))
            for hf in range(2):
                rows = (hf, pl.ds(p * 4, NC, stride=SP), slice(None))
                stores += [(sre[g % 3], rows, s[hf * NC:(hf + 1) * NC, 0:128]),
                           (sim[g % 3], rows, s[hf * NC:(hf + 1) * NC, 128:256])]
        g, p = item(T_INTRA + LMM)
        if g is not None:
            gg = g0 + g
            rows = (pl.ds(gg * 8 + p, NC, stride=YP), slice(None))
            stores.append((yp, rows, live.pop(("y", g % 3, p))))
        for ref, idx, val in stores:
            ref[idx] = val

    T0 = 8 * (-(-(T_INTRA + LMM) // 8))
    NJ = (8 * NG - T0) // SB
    live = {}
    for tau in range(T0):
        s4_slot(tau, 0, live)

    def grp_body(j, live):
        live = dict(live)
        for tau in range(T0, T0 + SB):
            s4_slot(tau, (SB // 8) * j, live)
        return live

    live = dict(lax.fori_loop(0, NJ, grp_body, live))
    for tau in range(T0 + SB * NJ, 8 * NG + T_INTRA + LMM):
        s4_slot(tau, 0, live)

    def s4_output(s):
        c, sb = s // 2, s % 2
        rows = pl.ds(pl.multiple_of(c * T, T), T)
        res = []
        xt = yp[pl.ds(c * YP + sb * 128, 128), :].T
        for hf in range(2):
            cols = pl.ds(pl.multiple_of(sb * 256 + hf * 128, 128), 128)
            res.append((rows, cols, xt[hf * T:(hf + 1) * T]))
        xt = yp[pl.ds(c * YP + (NB // 2) * 128 - 64, 128), :].T
        res.append((rows, pl.ds(D - 128, 128), jnp.where(lo64, pltpu.roll(xt[0:T], 64, 1), xt[T:2 * T])))
        return [(r, cl, (y + u_ref[r, cl].astype(F32) * dsk[:, cl]).astype(BF16)) for r, cl, y in res]

    for m, raw in enumerate((raw_q, raw_k, raw_v)):
        load_w[m].wait()

        def w_body(j, carry, m=m, src=raw.reshape(D // 2 * WP, Dh)):
            rows = pl.ds(pl.multiple_of(j * WB, WB), WB)
            cols = slice(m * Dh, (m + 1) * Dh)
            prev = None
            for i in range(H // 2 + 1):
                if i < H // 2:
                    cur = [src[pl.ds(j * WB * WP + i + o, WB, stride=WP), :] for o in (0, H // 2)]
                if prev is not None:
                    wqkv[2 * i - 2, rows, cols] = pltpu.pack_elementwise(prev, packed_dtype=jnp.uint16)
                    wqkv[2 * i - 1, rows, cols] = pltpu.pack_elementwise([x >> 16 for x in prev], packed_dtype=jnp.uint16)
                prev = cur
            return carry

        lax.fori_loop(0, D // 2 // WB, w_body, 0)
    load_wo.wait()

    load_x0.wait()
    load_x1.start()

    hbuf[0:M, :] = mem_ref[...].astype(F32)
    row = lax.broadcasted_iota(jnp.int32, (R, R), 0)
    col = lax.broadcasted_iota(jnp.int32, (R, R), 1)
    scale = Dh ** -0.5

    def seg_body(s, carry):
        r0 = pl.multiple_of(s * SEG, SEG)
        hbuf[M:R, :] = x_v[pl.ds(r0, SEG), :].astype(F32)
        mask = (row < M) | (row >= col)
        q, k, v, p, o = {}, {}, {}, {}, {}
        acc, h0, step = None, 0, 0
        while h0 < H:
            if step < H:
                r = _dot(hbuf[...], pltpu.bitcast(wqkv[step], BF16))
                q[step] = r[:, 0:Dh] * scale
                k[step] = r[:, Dh:2 * Dh].astype(BF16)
                v[step] = r[:, 2 * Dh:3 * Dh].astype(BF16)
            h = step - LQK
            if 0 <= h < H:
                sc = jnp.where(mask, _dot(q.pop(h), k.pop(h), _NT), -1e9)
                e = jnp.exp(sc - jnp.max(sc, axis=-1, keepdims=True))
                p[h] = e / jnp.sum(e, axis=-1, keepdims=True)
            h = step - LPV
            if 0 <= h < H:
                o[h] = _dot(p.pop(h), v.pop(h))
            h = h0 + GW - 1
            if h in o and (h <= step - LWO or step >= H):
                oo = jnp.concatenate([o.pop(i) for i in range(h0, h + 1)], axis=1)
                d = _dot(oo, pltpu.bitcast(wo[pl.ds(h0 * Dh // 2, GW * Dh // 2), :], BF16))
                acc = d if acc is None else acc + d
                h0 += GW
            if step == YSTEP:
                s4_out = s4_output(s)
            step += 1
        hbuf[0:M, :] = acc[0:M]
        ob[pl.ds(r0, SEG), D:2 * D] = acc[M:R].astype(BF16)
        for r, cl, y in s4_out:
            ob[r, cl] = y
        return carry

    def store(j):
        rows = pl.ds(pl.multiple_of(j * X0, X0), X0)
        return copy(ob.at[rows, :], o_hbm.at[rows, :], sems.at[7])

    def outer(j, carry):
        lax.fori_loop(j * PER, (j + 1) * PER, seg_body, 0)
        store(j).start()

        @pl.when(j == 0)
        def _():
            load_x1.wait()

        return carry

    lax.fori_loop(0, NO, outer, 0)
    copy(ob, o_hbm, sems.at[7]).wait()


@functools.partial(jax.jit, static_argnames=("B_seg_len",))
def pallas_concat_heads__ssm_conv_s4__memory_aug_recurrent_mem_tr__prompt_kernel(
    A_u, A_A_re, A_A_im, A_B_re, A_B_im, A_C_re, A_C_im, A_log_dt, A_Dskip,
    B_x, B_mem0, B_Wq, B_Wk, B_Wv, B_Wo, B_seg_len,
):
    Bsz, L, D = A_u.shape
    N = A_A_re.shape[1]
    _, H, Dh = B_Wq.shape
    M = B_mem0.shape[1]
    SEG = int(B_seg_len)
    assert SEG * 2 == T and D == 640 and Bsz == 1 and B_x.shape == A_u.shape and N == 128 and Dh == 128
    NC = L // T
    NB = D // 128

    vmem = pl.BlockSpec(memory_space=pltpu.VMEM)
    hbm = pl.BlockSpec(memory_space=pl.ANY)
    scratch = [
        pltpu.VMEM((D // 2, WP, Dh), U32), pltpu.VMEM((D // 2, WP, Dh), U32), pltpu.VMEM((D // 2, WP, Dh), U32),
        pltpu.VMEM((L, D), BF16),
        pltpu.VMEM((L, D), BF16),
        pltpu.VMEM((H, D // 2, 3 * Dh), U32),
        pltpu.VMEM((H * Dh // 2, D), U32),
        pltpu.VMEM((M + SEG, D), F32),
        pltpu.VMEM((L, 2 * D), BF16),
        pltpu.VMEM((2, (D + 1) * PP, N), F32),
        pltpu.VMEM((11, D, N), F32),
        pltpu.VMEM(((D // 2 + 1) * UP, 128), U32),
        pltpu.VMEM(((NC + 1) * YP, 128), F32),
        pltpu.VMEM((1, D), F32),
        pltpu.SemaphoreType.DMA((8,)),
    ] + 3 * [
        pltpu.VMEM((2, (NC + 1) * SP, N), F32),
        pltpu.VMEM((2, (NC + 1) * SP, N), F32),
        pltpu.VMEM((10 * ZP, N), U32),
        pltpu.VMEM((10 * ZP, N), U32),
        pltpu.VMEM((8, T, N), U32),
        pltpu.VMEM((8, T, N), U32),
    ]
    out = pl.pallas_call(
        functools.partial(_kernel, L=L, D=D, N=N, H=H, Dh=Dh, M=M, SEG=SEG),
        out_shape=jax.ShapeDtypeStruct((L, 2 * D), A_u.dtype),
        in_specs=[vmem] * 9 + [hbm] * 6,
        out_specs=hbm,
        scratch_shapes=scratch,
        compiler_params=pltpu.CompilerParams(vmem_limit_bytes=120 * 1024 * 1024),
        name="s4_rmt",
    )(A_A_re, A_A_im, A_B_re, A_B_im, A_C_re, A_C_im,
      A_log_dt, A_Dskip, B_mem0.reshape(M, D),
      A_u.reshape(L, D), B_x.reshape(L, D), B_Wq.reshape(D // 2, 2 * H, Dh), B_Wk.reshape(D // 2, 2 * H, Dh),
      B_Wv.reshape(D // 2, 2 * H, Dh), B_Wo.reshape(H * Dh, D))
    return out.reshape(Bsz, L, 2 * D)
```

```python
import functools

import jax
import jax.numpy as jnp
from jax import lax
import jax.experimental.pallas as pl
import jax.experimental.pallas.tpu as pltpu

F32 = jnp.float32
BF16 = jnp.bfloat16
U32 = jnp.uint32

LMM, T_STATE, T_SCAN, T_TAPS, T_INTRA = 2, 1, 12, 22, 30
SB = 144
WB = 32
PER = 2
UC = 16
YSTEP = 16
T = 64
LQK, LPV, LWO, GW = 2, 6, 16, 2

PP, UP, YP, SP, ZP, WP = 33, 17, 321, 33, 33, 40

_NN = (((1,), (0,)), ((), ()))
_NT = (((1,), (1,)), ((), ()))


def _dot(a, b, dims=_NN):
    return lax.dot_general(a, b, dims, preferred_element_type=F32)


def _pack(a, b):
    return pltpu.pack_elementwise([a, b], packed_dtype=BF16)


def _cmul(ar, ai, br, bi):
    return ar * br - ai * bi, ar * bi + ai * br


def _kernel(are_ref, aim_ref, bre_ref, bim_ref, cre_ref, cim_ref, ldt_ref, dsk_ref,
            mem_ref, u_hbm, x_hbm, wq_hbm, wk_hbm, wv_hbm, wo_hbm,
            o_hbm,
            raw_q, raw_k, raw_v, u_ref, x_v, wqkv, wo, ob,
            pw, cst, up, yp, dsk, sems, *slots,
            L, D, N, H, Dh, M, SEG):
    sre, sim, zre, zim, tre, tim = (slots[i::6] for i in range(6))
    NC = L // T
    NB = D // 128
    NSEG = L // SEG
    R = M + SEG

    NO = NSEG // PER
    X0 = PER * SEG
    copy = pltpu.make_async_copy
    load_u = copy(u_hbm, u_ref, sems.at[0])
    load_w = [copy(w.bitcast(U32), r.at[:, pl.ds(0, H), :], sems.at[1 + i])
              for i, (w, r) in enumerate(((wq_hbm, raw_q), (wk_hbm, raw_k), (wv_hbm, raw_v)))]
    load_wo = copy(wo_hbm.bitcast(U32), wo, sems.at[4])
    load_x0 = copy(x_hbm.at[pl.ds(0, X0), :], x_v.at[pl.ds(0, X0), :], sems.at[5])
    load_x1 = copy(x_hbm.at[pl.ds(X0, L - X0), :], x_v.at[pl.ds(X0, L - X0), :], sems.at[6])
    for c in [load_u] + load_w + [load_wo, load_x0]:
        c.start()

    lane = lax.broadcasted_iota(jnp.int32, (T, 128), 1)
    lo64 = lane < 64
    lo32 = lax.broadcasted_iota(jnp.int32, (NC, 128), 1) < 64

    ldt = ldt_ref[...].astype(F32).reshape(1, D)
    dsk[...] = dsk_ref[...].astype(F32).reshape(1, D)
    for b in range(NB):
        rows = slice(b * 128, (b + 1) * 128)
        dt = jnp.exp(ldt[:, rows])
        dt = jnp.broadcast_to(dt, (128, 128)).T
        a = dt * are_ref[rows, :].astype(F32)
        th = dt * aim_ref[rows, :].astype(F32)
        ea = jnp.exp(a)
        w = (ea * jnp.cos(th), ea * jnp.sin(th))
        c = _cmul(cre_ref[rows, :].astype(F32), cim_ref[rows, :].astype(F32),
                  dt * bre_ref[rows, :].astype(F32), dt * bim_ref[rows, :].astype(F32))
        g = _cmul(*c, *w)
        p = {0: (jnp.ones_like(ea), jnp.zeros_like(ea)), 1: _cmul(*w, *w)}
        p[2] = _cmul(*p[1], *p[1])
        p[3] = _cmul(*p[2], *p[1])
        p[4] = _cmul(*p[2], *p[2])
        p[5] = _cmul(*p[4], *p[1])
        p[6] = _cmul(*p[4], *p[2])
        p[7] = _cmul(*p[4], *p[3])
        w16 = _cmul(*p[4], *p[4])
        w32 = _cmul(*w16, *w16)
        w64 = _cmul(*w32, *w32)
        for ri in range(2):
            for j in range(8):
                pw[ri, pl.ds(b * 128 * PP + j * 4, 128, stride=PP), :] = p[j][ri]
            cst[0 + ri, rows, :] = w[ri]
            cst[2 + ri, rows, :] = w16[ri]
            cst[4 + ri, rows, :] = w64[ri]
            cst[6 + ri, rows, :] = g[ri]
        cst[8, rows, :] = -g[0]
        cst[9, rows, :] = c[0]
        cst[10, rows, :] = -c[1]

    flip = jnp.where(lax.broadcasted_iota(jnp.int32, (T, T), 0)
                     + lax.broadcasted_iota(jnp.int32, (T, T), 1) == T - 1, 1.0, 0.0).astype(BF16)
    load_u.wait()

    def u_body(j, carry):
        cs = [j * UC + i for i in range(UC)]
        ns = [_dot(flip, u_ref[pl.ds(pl.multiple_of(c * T, T), T), :]) for c in cs]
        ns = [_pack(ns[i], ns[i + 1]) for i in range(0, UC, 2)]
        cs = [j * (UC // 2) + i for i in range(UC // 2)]
        stores = []
        for c, n in zip(cs, ns):
            for sb in range(NB // 2):
                xt = jnp.concatenate([n[:, sb * 256:sb * 256 + 128], n[:, sb * 256 + 128:sb * 256 + 256]], axis=0).T
                stores.append((pl.ds(sb * 128 * UP + c, 128, stride=UP), xt))
        if NB % 2:
            for i in range(0, UC // 2, 2):
                n0, n1 = ns[i][:, D - 128:], ns[i + 1][:, D - 128:]
                top = jnp.where(lo64, n0, pltpu.roll(n1, 64, 1))
                bot = jnp.where(lo64, pltpu.roll(n0, 64, 1), n1)
                xt = jnp.concatenate([top, bot], axis=0).T
                for cc in range(2):
                    stores.append((pl.ds((NB // 2) * 128 * UP + cs[i + cc], 64, stride=UP), xt[cc * 64:(cc + 1) * 64]))
        for rows, val in stores:
            up[rows, :] = val
        return carry

    lax.fori_loop(0, NC // UC, u_body, 0)

    r2 = 2 * lax.broadcasted_iota(jnp.int32, (T // 2, 128), 0)
    l2 = lax.broadcasted_iota(jnp.int32, (T // 2, 128), 1)
    hank_ok = (l2 % T) + r2 >= T - 2
    hank_idx = jnp.where(hank_ok, l2 + r2 - (T - 2), l2)
    lane8 = lax.broadcasted_iota(jnp.int32, (8, 128), 1)
    not_k = lax.broadcasted_iota(jnp.int32, (8, 128), 0) != 0

    def chans(g):
        ca = (g // 16) * 256 + (g % 16) * 8
        ch = [ca, ca + 128 - 64 * (g // (16 * (NB // 2)))]
        return ch if isinstance(g, int) else [pl.multiple_of(c, 8) for c in ch]

    def lhs(g, p):
        x = pltpu.bitcast(up[pl.ds((g * 8 + p) * UP, NC // 2), :], BF16)
        return jnp.concatenate([jnp.where(lo32, x, 0.0), jnp.where(lo32, 0.0, x)], axis=0)

    NG = D // 16

    def s4_slot(tau, g0, live):
        def item(lag):
            g, p = divmod(tau - lag, 8)
            return (g, p) if 0 <= g < NG else (None, None)

        stores = []
        g, p = item(T_STATE)
        if g is not None:
            tr, ti = live.pop(("v", g % 3, p))
            live["s", g % 3, p] = _dot(lhs(g0 + g, p), pltpu.bitcast(jnp.concatenate([tr, ti], axis=1), BF16))
            stores += [(tre[g % 3], (p,), tr), (tim[g % 3], (p,), ti)]
        g, p = item(T_TAPS)
        if g is not None:
            rows = pl.ds(p * ZP, NC)
            y = (_dot(pltpu.bitcast(zre[g % 3][rows, :], BF16), pltpu.bitcast(tre[g % 3][p], BF16), _NT)
                 + _dot(pltpu.bitcast(zim[g % 3][rows, :], BF16), pltpu.bitcast(tim[g % 3][p], BF16), _NT))
            k2 = jnp.where(lane8 < 64, y[0:8], y[NC:NC + 8])
            k1 = jnp.where(lane8 % T == 0, 0.0, pltpu.roll(k2, 1, 1))
            kq = _pack(k1, k2)
            kq = jnp.broadcast_to(kq[0:1, :], (T // 2, 128))
            live["h", g % 3, p] = jnp.where(hank_ok, jnp.take_along_axis(kq, hank_idx, axis=1), U32(0))
            live["y", g % 3, p] = jnp.concatenate(
                [jnp.where(not_k, k2, 0.0), jnp.where(lo32[8:], y[8:NC], y[NC + 8:])], axis=0)
        g, p = item(T_INTRA)
        if g is not None:
            hk = live.pop(("h", g % 3, p))
            y = _dot(lhs(g0 + g, p), pltpu.bitcast(jnp.concatenate([hk, hk], axis=0), BF16))
            live["y", g % 3, p] = live["y", g % 3, p] + jnp.where(lo32, y[0:NC], y[NC:2 * NC])
        g, p = item(0)
        if g is not None:
            ch = chans(g0 + g)
            vr, vi = [], []
            for hf in range(2):
                base = pl.ds((ch[hf] + p) * PP, 8, stride=4)
                ev = (pw[0, base, :], pw[1, base, :])
                bc = [jnp.broadcast_to(cst[n, pl.ds(ch[hf] + p, 1), :], (8, 128)) for n in range(4)]
                od = _cmul(*ev, bc[0], bc[1])
                for k in range(T // 16):
                    vr.append(_pack(ev[0], od[0]))
                    vi.append(_pack(ev[1], od[1]))
                    if k + 1 < T // 16:
                        ev = _cmul(*ev, bc[2], bc[3])
                        od = _cmul(*od, bc[2], bc[3])
            live["v", g % 3, p] = (jnp.concatenate(vr, axis=0), jnp.concatenate(vi, axis=0))
        g, p = item(T_SCAN + 1)
        if g is not None:
            for (hf, c), (zr, zi) in live.pop(("z", g % 3, p)).items():
                rows = (pl.ds((hf * NC + c) // 2, 8, stride=ZP), slice(None))
                stores += [(zre[g % 3], rows, zr), (zim[g % 3], rows, zi)]
        g, p = item(T_SCAN)
        if g is not None:
            ch = chans(g0 + g)
            z = {}
            for hf in range(2):
                wtr, wti, gr, gi, ngr = [cst[4 + n, pl.ds(ch[hf], 8), :] for n in range(5)]
                if p == 0:
                    live["e", hf] = (cst[9, pl.ds(ch[hf], 8), :], cst[10, pl.ds(ch[hf], 8), :])
                for c in range(p * NC // 8, min((p + 1) * NC // 8, NC - 1)):
                    rows = pl.ds(c * SP, 8, stride=4)
                    xr, xi = sre[g % 3][hf, rows, :], sim[g % 3][hf, rows, :]
                    if c > 0:
                        pr, pi = _cmul(*live["x", hf], wtr, wti)
                        xr, xi = pr + xr, pi + xi
                    live["x", hf] = (xr, xi)
                    zn = (xr * gr - xi * gi, xi * ngr - xr * gi)
                    if c % 2:
                        live["e", hf] = zn
                    else:
                        z[hf, c] = [_pack(a, b) for a, b in zip(live.pop(("e", hf)), zn)]
            live["z", g % 3, p] = z
        g, p = item(T_STATE + LMM)
        if g is not None:
            s = live.pop(("s", g % 3, p))
            for hf in range(2):
                rows = (hf, pl.ds(p * 4, NC, stride=SP), slice(None))
                stores += [(sre[g % 3], rows, s[hf * NC:(hf + 1) * NC, 0:128]),
                           (sim[g % 3], rows, s[hf * NC:(hf + 1) * NC, 128:256])]
        g, p = item(T_INTRA + LMM)
        if g is not None:
            gg = g0 + g
            rows = (pl.ds(gg * 8 + p, NC, stride=YP), slice(None))
            stores.append((yp, rows, live.pop(("y", g % 3, p))))
        for ref, idx, val in stores:
            ref[idx] = val

    T0 = 8 * (-(-(T_INTRA + LMM) // 8))
    NJ = (8 * NG - T0) // SB
    live = {}
    for tau in range(T0):
        s4_slot(tau, 0, live)

    def grp_body(j, live):
        live = dict(live)
        for tau in range(T0, T0 + SB):
            s4_slot(tau, (SB // 8) * j, live)
        return live

    live = dict(lax.fori_loop(0, NJ, grp_body, live))
    for tau in range(T0 + SB * NJ, 8 * NG + T_INTRA + LMM):
        s4_slot(tau, 0, live)

    def s4_output(s):
        c, sb = s // 2, s % 2
        rows = pl.ds(pl.multiple_of(c * T, T), T)
        res = []
        xt = yp[pl.ds(c * YP + sb * 128, 128), :].T
        for hf in range(2):
            cols = pl.ds(pl.multiple_of(sb * 256 + hf * 128, 128), 128)
            res.append((rows, cols, xt[hf * T:(hf + 1) * T]))
        xt = yp[pl.ds(c * YP + (NB // 2) * 128 - 64, 128), :].T
        res.append((rows, pl.ds(D - 128, 128), jnp.where(lo64, pltpu.roll(xt[0:T], 64, 1), xt[T:2 * T])))
        return [(r, cl, (y + u_ref[r, cl].astype(F32) * dsk[:, cl]).astype(BF16)) for r, cl, y in res]

    for m, raw in enumerate((raw_q, raw_k, raw_v)):
        load_w[m].wait()

        def w_body(j, carry, m=m, src=raw.reshape(D // 2 * WP, Dh)):
            rows = pl.ds(pl.multiple_of(j * WB, WB), WB)
            cols = slice(m * Dh, (m + 1) * Dh)
            prev = None
            for i in range(H // 2 + 1):
                if i < H // 2:
                    cur = [src[pl.ds(j * WB * WP + i + o, WB, stride=WP), :] for o in (0, H // 2)]
                if prev is not None:
                    wqkv[2 * i - 2, rows, cols] = pltpu.pack_elementwise(prev, packed_dtype=jnp.uint16)
                    wqkv[2 * i - 1, rows, cols] = pltpu.pack_elementwise([x >> 16 for x in prev], packed_dtype=jnp.uint16)
                prev = cur
            return carry

        lax.fori_loop(0, D // 2 // WB, w_body, 0)
    load_wo.wait()

    load_x0.wait()
    load_x1.start()

    row = lax.broadcasted_iota(jnp.int32, (R, R), 0)
    col = lax.broadcasted_iota(jnp.int32, (R, R), 1)
    scale = Dh ** -0.5

    def flush(stores):
        for r, cl, y in stores:
            ob[r, cl] = y

    def segment(s, mem, pending):
        r0 = pl.multiple_of(s * SEG, SEG)
        hid = jnp.concatenate([mem, x_v[pl.ds(r0, SEG), :].astype(F32)], axis=0)
        mask = (row < M) | (row >= col)
        q, k, v, p, o = {}, {}, {}, {}, {}
        acc, h0, step = None, 0, 0
        while h0 < H:
            if step < H:
                r = _dot(hid, pltpu.bitcast(wqkv[step], BF16))
                q[step] = r[:, 0:Dh] * scale
                k[step] = r[:, Dh:2 * Dh].astype(BF16)
                v[step] = r[:, 2 * Dh:3 * Dh].astype(BF16)
            h = step - LQK
            if 0 <= h < H:
                sc = jnp.where(mask, _dot(q.pop(h), k.pop(h), _NT), -1e9)
                e = jnp.exp(sc - jnp.max(sc, axis=-1, keepdims=True))
                p[h] = e / jnp.sum(e, axis=-1, keepdims=True)
            h = step - LPV
            if 0 <= h < H:
                o[h] = _dot(p.pop(h), v.pop(h))
            h = h0 + GW - 1
            if h in o and (h <= step - LWO or step >= H):
                oo = jnp.concatenate([o.pop(i) for i in range(h0, h + 1)], axis=1)
                d = _dot(oo, pltpu.bitcast(wo[pl.ds(h0 * Dh // 2, GW * Dh // 2), :], BF16))
                acc = d if acc is None else acc + d
                h0 += GW
            if step == 2:
                flush(pending)
            if step == YSTEP:
                s4_out = s4_output(s)
            if step == YSTEP + 4:
                flush(s4_out)
            step += 1
        return acc[0:M], [(pl.ds(r0, SEG), slice(D, 2 * D), acc[M:R].astype(BF16))]

    def store(j):
        rows = pl.ds(pl.multiple_of(j * X0, X0), X0)
        return copy(ob.at[rows, :], o_hbm.at[rows, :], sems.at[7])

    def outer(j, mem):
        pending = []
        for i in range(PER):
            mem, pending = segment(j * PER + i, mem, pending)
        flush(pending)
        store(j).start()

        @pl.when(j == 0)
        def _():
            load_x1.wait()

        return mem

    lax.fori_loop(0, NO, outer, mem_ref[...].astype(F32))
    copy(ob, o_hbm, sems.at[7]).wait()


@functools.partial(jax.jit, static_argnames=("B_seg_len",))
def pallas_concat_heads__ssm_conv_s4__memory_aug_recurrent_mem_tr__prompt_kernel(
    A_u, A_A_re, A_A_im, A_B_re, A_B_im, A_C_re, A_C_im, A_log_dt, A_Dskip,
    B_x, B_mem0, B_Wq, B_Wk, B_Wv, B_Wo, B_seg_len,
):
    Bsz, L, D = A_u.shape
    N = A_A_re.shape[1]
    _, H, Dh = B_Wq.shape
    M = B_mem0.shape[1]
    SEG = int(B_seg_len)
    assert SEG * 2 == T and D == 640 and Bsz == 1 and B_x.shape == A_u.shape and N == 128 and Dh == 128
    NC = L // T
    NB = D // 128

    vmem = pl.BlockSpec(memory_space=pltpu.VMEM)
    hbm = pl.BlockSpec(memory_space=pl.ANY)
    scratch = [
        pltpu.VMEM((D // 2, WP, Dh), U32), pltpu.VMEM((D // 2, WP, Dh), U32), pltpu.VMEM((D // 2, WP, Dh), U32),
        pltpu.VMEM((L, D), BF16),
        pltpu.VMEM((L, D), BF16),
        pltpu.VMEM((H, D // 2, 3 * Dh), U32),
        pltpu.VMEM((H * Dh // 2, D), U32),
        pltpu.VMEM((L, 2 * D), BF16),
        pltpu.VMEM((2, (D + 1) * PP, N), F32),
        pltpu.VMEM((11, D, N), F32),
        pltpu.VMEM(((D // 2 + 1) * UP, 128), U32),
        pltpu.VMEM(((NC + 1) * YP, 128), F32),
        pltpu.VMEM((1, D), F32),
        pltpu.SemaphoreType.DMA((8,)),
    ] + 3 * [
        pltpu.VMEM((2, (NC + 1) * SP, N), F32),
        pltpu.VMEM((2, (NC + 1) * SP, N), F32),
        pltpu.VMEM((10 * ZP, N), U32),
        pltpu.VMEM((10 * ZP, N), U32),
        pltpu.VMEM((8, T, N), U32),
        pltpu.VMEM((8, T, N), U32),
    ]
    out = pl.pallas_call(
        functools.partial(_kernel, L=L, D=D, N=N, H=H, Dh=Dh, M=M, SEG=SEG),
        out_shape=jax.ShapeDtypeStruct((L, 2 * D), A_u.dtype),
        in_specs=[vmem] * 9 + [hbm] * 6,
        out_specs=hbm,
        scratch_shapes=scratch,
        compiler_params=pltpu.CompilerParams(vmem_limit_bytes=120 * 1024 * 1024),
        name="s4_rmt",
    )(A_A_re, A_A_im, A_B_re, A_B_im, A_C_re, A_C_im,
      A_log_dt, A_Dskip, B_mem0.reshape(M, D),
      A_u.reshape(L, D), B_x.reshape(L, D), B_Wq.reshape(D // 2, 2 * H, Dh), B_Wk.reshape(D // 2, 2 * H, Dh),
      B_Wv.reshape(D // 2, 2 * H, Dh), B_Wo.reshape(H * Dh, D))
    return out.reshape(Bsz, L, 2 * D)
```

```python
import functools

import jax
import jax.numpy as jnp
from jax import lax
import jax.experimental.pallas as pl
import jax.experimental.pallas.tpu as pltpu

F32 = jnp.float32
BF16 = jnp.bfloat16
U32 = jnp.uint32

LMM, T_STATE, T_SCAN, T_TAPS, T_INTRA = 2, 1, 12, 22, 30
SB = 144
WB = 32
PER = 2
UC = 16
YSTEP = 16
T = 64
LQK, LPV, LWO, GW = 2, 6, 16, 2

PP, UP, YP, SP, ZP, WP = 33, 17, 321, 33, 33, 40

_NN = (((1,), (0,)), ((), ()))
_NT = (((1,), (1,)), ((), ()))


def _dot(a, b, dims=_NN):
    return lax.dot_general(a, b, dims, preferred_element_type=F32)


def _pack(a, b):
    return pltpu.pack_elementwise([a, b], packed_dtype=BF16)


def _cmul(ar, ai, br, bi):
    return ar * br - ai * bi, ar * bi + ai * br


def _csqrt(re, im):
    m = jnp.maximum(jnp.abs(re), jnp.abs(im))
    nz = m > 0
    inv = 1.0 / jnp.where(nz, m, 1.0)
    a, b = jnp.where(nz, re * inv, 1.0), im * inv
    r2 = a * a + b * b
    t2 = 0.5 * (r2 * lax.rsqrt(r2) + jnp.abs(a))
    rs = lax.rsqrt(t2)
    big, small = t2 * rs, 0.5 * b * rs
    sm = jnp.sqrt(m)
    return jnp.where(a >= 0, big, small) * sm, jnp.where(a >= 0, small, big) * sm


def _kernel(are_ref, aim_ref, bre_ref, bim_ref, cre_ref, cim_ref, ldt_ref, dsk_ref,
            mem_ref, u_hbm, x_hbm, wq_hbm, wk_hbm, wv_hbm, wo_hbm,
            o_hbm,
            raw_q, raw_k, raw_v, u_ref, x_v, wqkv, wo, ob,
            pw, cst, up, yp, dsk, sems, *slots,
            L, D, N, H, Dh, M, SEG):
    sre, sim, zre, zim, tre, tim = (slots[i::6] for i in range(6))
    NC = L // T
    NB = D // 128
    NSEG = L // SEG
    R = M + SEG

    NO = NSEG // PER
    X0 = PER * SEG
    copy = pltpu.make_async_copy
    load_u = copy(u_hbm, u_ref.at[pl.ds(0, L), :], sems.at[0])
    load_w = [copy(w.bitcast(U32), r.at[:, pl.ds(0, H), :], sems.at[1 + i])
              for i, (w, r) in enumerate(((wq_hbm, raw_q), (wk_hbm, raw_k), (wv_hbm, raw_v)))]
    load_wo = copy(wo_hbm.bitcast(U32), wo, sems.at[4])
    load_x0 = copy(x_hbm.at[pl.ds(0, X0), :], x_v.at[pl.ds(0, X0), :], sems.at[5])
    load_x1 = copy(x_hbm.at[pl.ds(X0, L - X0), :], x_v.at[pl.ds(X0, L - X0), :], sems.at[6])
    for c in [load_u] + load_w + [load_wo, load_x0]:
        c.start()

    lane = lax.broadcasted_iota(jnp.int32, (T, 128), 1)
    lo64 = lane < 64
    lo32 = lax.broadcasted_iota(jnp.int32, (NC, 128), 1) < 64

    ldt = ldt_ref[...].astype(F32).reshape(1, D)
    dsk[...] = dsk_ref[...].astype(F32).reshape(1, D)
    for b in range(NB):
        rows = slice(b * 128, (b + 1) * 128)
        dt = jnp.exp(ldt[:, rows])
        dt = jnp.broadcast_to(dt, (128, 128)).T
        a = dt * are_ref[rows, :].astype(F32)
        th = dt * aim_ref[rows, :].astype(F32)
        ea = jnp.exp(a)
        w = (ea * jnp.cos(th), ea * jnp.sin(th))
        c = _cmul(cre_ref[rows, :].astype(F32), cim_ref[rows, :].astype(F32),
                  dt * bre_ref[rows, :].astype(F32), dt * bim_ref[rows, :].astype(F32))
        sq = [w]
        for _ in range(6):
            sq.append(_cmul(*sq[-1], *sq[-1]))
        p = [_csqrt(*c)]
        for i in (1, 2, 3):
            p += [_cmul(*x, *sq[i]) for x in p]
        for ri in range(2):
            for j in range(8):
                pw[ri, pl.ds(b * 128 * PP + j * 4, 128, stride=PP), :] = p[j][ri]
            for n, x in enumerate((w, sq[4], sq[6], p[0])):
                cst[2 * n + ri, rows, :] = x[ri]

    flip = jnp.where(lax.broadcasted_iota(jnp.int32, (T, 2 * T), 0)
                     + lax.broadcasted_iota(jnp.int32, (T, 2 * T), 1) == T, 1.0, 0.0).astype(BF16)
    load_u.wait()
    u_ref[L:L + T, :] = jnp.zeros((T, D), BF16)
    u0 = u_ref[0:16, :].astype(F32)[0:1]
    for b in range(NB):
        rows = slice(b * 128, (b + 1) * 128)
        cst[8, rows, :] = jnp.broadcast_to(u0[:, rows], (128, 128)).T

    def u_body(j, carry):
        cs = [j * UC + i for i in range(UC)]
        ns = [_dot(flip, u_ref[pl.ds(pl.multiple_of(c * T, T), 2 * T), :]) for c in cs]
        ns = [_pack(ns[i], ns[i + 1]) for i in range(0, UC, 2)]
        cs = [j * (UC // 2) + i for i in range(UC // 2)]
        stores = []
        for c, n in zip(cs, ns):
            for sb in range(NB // 2):
                xt = jnp.concatenate([n[:, sb * 256:sb * 256 + 128], n[:, sb * 256 + 128:sb * 256 + 256]], axis=0).T
                stores.append((pl.ds(sb * 128 * UP + c, 128, stride=UP), xt))
        if NB % 2:
            for i in range(0, UC // 2, 2):
                n0, n1 = ns[i][:, D - 128:], ns[i + 1][:, D - 128:]
                top = jnp.where(lo64, n0, pltpu.roll(n1, 64, 1))
                bot = jnp.where(lo64, pltpu.roll(n0, 64, 1), n1)
                xt = jnp.concatenate([top, bot], axis=0).T
                for cc in range(2):
                    stores.append((pl.ds((NB // 2) * 128 * UP + cs[i + cc], 64, stride=UP), xt[cc * 64:(cc + 1) * 64]))
        for rows, val in stores:
            up[rows, :] = val
        return carry

    lax.fori_loop(0, NC // UC, u_body, 0)

    r2 = 2 * lax.broadcasted_iota(jnp.int32, (T // 2, 128), 0)
    l2 = lax.broadcasted_iota(jnp.int32, (T // 2, 128), 1)
    hank_ok = (l2 % T) + r2 >= T - 1
    hank_idx = jnp.where(hank_ok, l2 + r2 - (T - 1), l2)
    hank_lo, hank_hi = hank_ok & (l2 < T), hank_ok & (l2 >= T)
    lane8 = lax.broadcasted_iota(jnp.int32, (8, 128), 1)
    not_k = lax.broadcasted_iota(jnp.int32, (8, 128), 0) != 0

    def chans(g):
        ca = (g // 16) * 256 + (g % 16) * 8
        ch = [ca, ca + 128 - 64 * (g // (16 * (NB // 2)))]
        return ch if isinstance(g, int) else [pl.multiple_of(c, 8) for c in ch]

    def lhs(g, p):
        return pltpu.bitcast(up[pl.ds((g * 8 + p) * UP, NC // 2), :], BF16)

    NG = D // 16

    def s4_slot(tau, g0, live):
        def item(lag):
            g, p = divmod(tau - lag, 8)
            return (g, p) if 0 <= g < NG else (None, None)

        stores = []
        g, p = item(T_STATE)
        if g is not None:
            tr, ti = live.pop(("v", g % 3, p))
            x = lhs(g0 + g, p)
            x = jnp.concatenate([jnp.where(lo32, x, 0.0), jnp.where(lo32, 0.0, x)], axis=0)
            live["s", g % 3, p] = _dot(x, pltpu.bitcast(jnp.concatenate([tr, ti], axis=1), BF16))
            stores += [(tre[g % 3], (p,), tr), (tim[g % 3], (p,), ti)]
        g, p = item(T_TAPS)
        if g is not None:
            rows = pl.ds(p * ZP, NC)
            y = (_dot(pltpu.bitcast(zre[g % 3][rows, :], BF16), pltpu.bitcast(tre[g % 3][p], BF16), _NT)
                 - _dot(pltpu.bitcast(zim[g % 3][rows, :], BF16), pltpu.bitcast(tim[g % 3][p], BF16), _NT))
            k2 = jnp.where(lane8 < 64, y[0:8], y[NC:NC + 8])
            k1 = jnp.where(lane8 % T == 0, 0.0, pltpu.roll(k2, 1, 1))
            kq = _pack(k1, k2)
            kq = jnp.broadcast_to(kq[0:1, :], (T // 2, 128))
            live["h", g % 3, p] = jnp.take_along_axis(kq, hank_idx, axis=1)
            first = jnp.where(lane8 < 64, *[jnp.broadcast_to(cst[8, pl.ds(c + p, 1), :], (8, 128)) for c in chans(g0 + g)])
            live["y", g % 3, p] = jnp.concatenate(
                [jnp.where(not_k, k2, k2 * first), jnp.where(lo32[8:], y[8:NC], y[NC + 8:])], axis=0)
        g, p = item(T_INTRA)
        if g is not None:
            hk = live.pop(("h", g % 3, p))
            hk = jnp.concatenate([jnp.where(hank_lo, hk, U32(0)), jnp.where(hank_hi, hk, U32(0))], axis=0)
            live["y", g % 3, p] = live["y", g % 3, p] + _dot(lhs(g0 + g, p), pltpu.bitcast(hk, BF16))
        g, p = item(0)
        if g is not None:
            ch = chans(g0 + g)
            vr, vi = [], []
            for hf in range(2):
                base = pl.ds((ch[hf] + p) * PP, 8, stride=4)
                ev = (pw[0, base, :], pw[1, base, :])
                bc = [jnp.broadcast_to(cst[n, pl.ds(ch[hf] + p, 1), :], (8, 128)) for n in range(4)]
                od = _cmul(*ev, bc[0], bc[1])
                for k in range(T // 16):
                    vr.append(_pack(ev[0], od[0]))
                    vi.append(_pack(ev[1], od[1]))
                    if k + 1 < T // 16:
                        ev = _cmul(*ev, bc[2], bc[3])
                        od = _cmul(*od, bc[2], bc[3])
            live["v", g % 3, p] = (jnp.concatenate(vr, axis=0), jnp.concatenate(vi, axis=0))
        g, p = item(T_SCAN + 1)
        if g is not None:
            for (hf, c), (zr, zi) in live.pop(("z", g % 3, p)).items():
                rows = (pl.ds((hf * NC + c) // 2, 8, stride=ZP), slice(None))
                stores += [(zre[g % 3], rows, zr), (zim[g % 3], rows, zi)]
        g, p = item(T_SCAN)
        if g is not None:
            ch = chans(g0 + g)
            z = {}
            for hf in range(2):
                wtr, wti = [cst[4 + n, pl.ds(ch[hf], 8), :] for n in range(2)]
                if p == 0:
                    live["e", hf] = [cst[6 + n, pl.ds(ch[hf], 8), :] for n in range(2)]
                    live["x", hf] = [x * cst[8, pl.ds(ch[hf], 8), :] for x in live["e", hf]]
                for c in range(p * NC // 8, min((p + 1) * NC // 8, NC - 1)):
                    rows = pl.ds(c * SP, 8, stride=4)
                    xr, xi = sre[g % 3][hf, rows, :], sim[g % 3][hf, rows, :]
                    pr, pi = _cmul(*live["x", hf], wtr, wti)
                    zn = live["x", hf] = [pr + xr, pi + xi]
                    if c % 2:
                        live["e", hf] = zn
                    else:
                        z[hf, c] = [_pack(a, b) for a, b in zip(live.pop(("e", hf)), zn)]
            live["z", g % 3, p] = z
        g, p = item(T_STATE + LMM)
        if g is not None:
            s = live.pop(("s", g % 3, p))
            for hf in range(2):
                rows = (hf, pl.ds(p * 4, NC, stride=SP), slice(None))
                stores += [(sre[g % 3], rows, s[hf * NC:(hf + 1) * NC, 0:128]),
                           (sim[g % 3], rows, s[hf * NC:(hf + 1) * NC, 128:256])]
        g, p = item(T_INTRA + LMM)
        if g is not None:
            gg = g0 + g
            rows = (pl.ds(gg * 8 + p, NC, stride=YP), slice(None))
            stores.append((yp, rows, live.pop(("y", g % 3, p))))
        for ref, idx, val in stores:
            ref[idx] = val

    T0 = 8 * (-(-(T_INTRA + LMM) // 8))
    NJ = (8 * NG - T0) // SB
    live = {}
    for tau in range(T0):
        s4_slot(tau, 0, live)

    def grp_body(j, live):
        live = dict(live)
        for tau in range(T0, T0 + SB):
            s4_slot(tau, (SB // 8) * j, live)
        return live

    live = dict(lax.fori_loop(0, NJ, grp_body, live))
    for tau in range(T0 + SB * NJ, 8 * NG + T_INTRA + LMM):
        s4_slot(tau, 0, live)

    def s4_output(s):
        c, sb = s // 2, s % 2
        rows = pl.ds(pl.multiple_of(c * T, T), T)
        res = []
        xt = yp[pl.ds(c * YP + sb * 128, 128), :].T
        for hf in range(2):
            cols = pl.ds(pl.multiple_of(sb * 256 + hf * 128, 128), 128)
            res.append((rows, cols, xt[hf * T:(hf + 1) * T]))
        xt = yp[pl.ds(c * YP + (NB // 2) * 128 - 64, 128), :].T
        res.append((rows, pl.ds(D - 128, 128), jnp.where(lo64, pltpu.roll(xt[0:T], 64, 1), xt[T:2 * T])))
        return [(r, cl, (y + u_ref[r, cl].astype(F32) * dsk[:, cl]).astype(BF16)) for r, cl, y in res]

    for m, raw in enumerate((raw_q, raw_k, raw_v)):
        load_w[m].wait()

        def w_body(j, carry, m=m, src=raw.reshape(D // 2 * WP, Dh)):
            rows = pl.ds(pl.multiple_of(j * WB, WB), WB)
            cols = slice(m * Dh, (m + 1) * Dh)
            prev = None
            for i in range(H // 2 + 1):
                if i < H // 2:
                    cur = [src[pl.ds(j * WB * WP + i + o, WB, stride=WP), :] for o in (0, H // 2)]
                if prev is not None:
                    wqkv[2 * i - 2, rows, cols] = pltpu.pack_elementwise(prev, packed_dtype=jnp.uint16)
                    wqkv[2 * i - 1, rows, cols] = pltpu.pack_elementwise([x >> 16 for x in prev], packed_dtype=jnp.uint16)
                prev = cur
            return carry

        lax.fori_loop(0, D // 2 // WB, w_body, 0)
    load_wo.wait()

    load_x0.wait()
    load_x1.start()

    row = lax.broadcasted_iota(jnp.int32, (R, R), 0)
    col = lax.broadcasted_iota(jnp.int32, (R, R), 1)
    scale = Dh ** -0.5

    def flush(stores):
        for r, cl, y in stores:
            ob[r, cl] = y

    def segment(s, mem, pending):
        r0 = pl.multiple_of(s * SEG, SEG)
        hid = jnp.concatenate([mem, x_v[pl.ds(r0, SEG), :].astype(F32)], axis=0)
        mask = (row < M) | (row >= col)
        q, k, v, p, o = {}, {}, {}, {}, {}
        acc, h0, step = None, 0, 0
        while h0 < H:
            if step < H:
                r = _dot(hid, pltpu.bitcast(wqkv[step], BF16))
                q[step] = r[:, 0:Dh] * scale
                k[step] = r[:, Dh:2 * Dh].astype(BF16)
                v[step] = r[:, 2 * Dh:3 * Dh].astype(BF16)
            h = step - LQK
            if 0 <= h < H:
                sc = jnp.where(mask, _dot(q.pop(h), k.pop(h), _NT), -1e9)
                e = jnp.exp(sc - jnp.max(sc, axis=-1, keepdims=True))
                p[h] = e / jnp.sum(e, axis=-1, keepdims=True)
            h = step - LPV
            if 0 <= h < H:
                o[h] = _dot(p.pop(h), v.pop(h))
            h = h0 + GW - 1
            if h in o and (h <= step - LWO or step >= H):
                oo = jnp.concatenate([o.pop(i) for i in range(h0, h + 1)], axis=1)
                d = _dot(oo, pltpu.bitcast(wo[pl.ds(h0 * Dh // 2, GW * Dh // 2), :], BF16))
                acc = d if acc is None else acc + d
                h0 += GW
            if step == 2:
                flush(pending)
            if step == YSTEP:
                s4_out = s4_output(s)
            if step == YSTEP + 4:
                flush(s4_out)
            step += 1
        return acc[0:M], [(pl.ds(r0, SEG), slice(D, 2 * D), acc[M:R].astype(BF16))]

    def store(j):
        rows = pl.ds(pl.multiple_of(j * X0, X0), X0)
        return copy(ob.at[rows, :], o_hbm.at[rows, :], sems.at[7])

    def outer(j, mem):
        pending = []
        for i in range(PER):
            mem, pending = segment(j * PER + i, mem, pending)
        flush(pending)
        store(j).start()

        @pl.when(j == 0)
        def _():
            load_x1.wait()

        return mem

    lax.fori_loop(0, NO, outer, mem_ref[...].astype(F32))
    copy(ob, o_hbm, sems.at[7]).wait()


@functools.partial(jax.jit, static_argnames=("B_seg_len",))
def pallas_concat_heads__ssm_conv_s4__memory_aug_recurrent_mem_tr__prompt_kernel(
    A_u, A_A_re, A_A_im, A_B_re, A_B_im, A_C_re, A_C_im, A_log_dt, A_Dskip,
    B_x, B_mem0, B_Wq, B_Wk, B_Wv, B_Wo, B_seg_len,
):
    Bsz, L, D = A_u.shape
    N = A_A_re.shape[1]
    _, H, Dh = B_Wq.shape
    M = B_mem0.shape[1]
    SEG = int(B_seg_len)
    assert SEG * 2 == T and D == 640 and Bsz == 1 and B_x.shape == A_u.shape and N == 128 and Dh == 128
    NC = L // T
    NB = D // 128

    vmem = pl.BlockSpec(memory_space=pltpu.VMEM)
    hbm = pl.BlockSpec(memory_space=pl.ANY)
    scratch = [
        pltpu.VMEM((D // 2, WP, Dh), U32), pltpu.VMEM((D // 2, WP, Dh), U32), pltpu.VMEM((D // 2, WP, Dh), U32),
        pltpu.VMEM((L + T, D), BF16),
        pltpu.VMEM((L, D), BF16),
        pltpu.VMEM((H, D // 2, 3 * Dh), U32),
        pltpu.VMEM((H * Dh // 2, D), U32),
        pltpu.VMEM((L, 2 * D), BF16),
        pltpu.VMEM((2, (D + 1) * PP, N), F32),
        pltpu.VMEM((9, D, N), F32),
        pltpu.VMEM(((D // 2 + 1) * UP, 128), U32),
        pltpu.VMEM(((NC + 1) * YP, 128), F32),
        pltpu.VMEM((1, D), F32),
        pltpu.SemaphoreType.DMA((8,)),
    ] + 3 * [
        pltpu.VMEM((2, (NC + 1) * SP, N), F32),
        pltpu.VMEM((2, (NC + 1) * SP, N), F32),
        pltpu.VMEM((10 * ZP, N), U32),
        pltpu.VMEM((10 * ZP, N), U32),
        pltpu.VMEM((8, T, N), U32),
        pltpu.VMEM((8, T, N), U32),
    ]
    out = pl.pallas_call(
        functools.partial(_kernel, L=L, D=D, N=N, H=H, Dh=Dh, M=M, SEG=SEG),
        out_shape=jax.ShapeDtypeStruct((L, 2 * D), A_u.dtype),
        in_specs=[vmem] * 9 + [hbm] * 6,
        out_specs=hbm,
        scratch_shapes=scratch,
        compiler_params=pltpu.CompilerParams(vmem_limit_bytes=120 * 1024 * 1024),
        name="s4_rmt",
    )(A_A_re, A_A_im, A_B_re, A_B_im, A_C_re, A_C_im,
      A_log_dt, A_Dskip, B_mem0.reshape(M, D),
      A_u.reshape(L, D), B_x.reshape(L, D), B_Wq.reshape(D // 2, 2 * H, Dh), B_Wk.reshape(D // 2, 2 * H, Dh),
      B_Wv.reshape(D // 2, 2 * H, Dh), B_Wo.reshape(H * Dh, D))
    return out.reshape(Bsz, L, 2 * D)
```

```python
import functools

import jax
import jax.numpy as jnp
from jax import lax
import jax.experimental.pallas as pl
import jax.experimental.pallas.tpu as pltpu

F32 = jnp.float32
BF16 = jnp.bfloat16
U32 = jnp.uint32

LMM, T_STATE, T_SCAN, T_TAPS, T_INTRA = 2, 1, 12, 22, 30
SB = 144
WB = 32
PER = 2
UC = 16
YSTEP = 16
T = 64
LQK, LPV, LWO, GW = 2, 6, 16, 2

PP, UP, YP, SP, ZP, WP = 33, 17, 321, 33, 33, 322

_NN = (((1,), (0,)), ((), ()))
_NT = (((1,), (1,)), ((), ()))


def _dot(a, b, dims=_NN):
    return lax.dot_general(a, b, dims, preferred_element_type=F32)


def _pack(a, b):
    return pltpu.pack_elementwise([a, b], packed_dtype=BF16)


def _cmul(ar, ai, br, bi):
    return ar * br - ai * bi, ar * bi + ai * br


def _csqrt(re, im):
    m = jnp.maximum(jnp.abs(re), jnp.abs(im))
    nz = m > 0
    inv = 1.0 / jnp.where(nz, m, 1.0)
    a, b = jnp.where(nz, re * inv, 1.0), im * inv
    r2 = a * a + b * b
    t2 = 0.5 * (r2 * lax.rsqrt(r2) + jnp.abs(a))
    rs = lax.rsqrt(t2)
    big, small = t2 * rs, 0.5 * b * rs
    sm = jnp.sqrt(m)
    return jnp.where(a >= 0, big, small) * sm, jnp.where(a >= 0, small, big) * sm


def _kernel(are_ref, aim_ref, bre_ref, bim_ref, cre_ref, cim_ref, ldt_ref, dsk_ref,
            mem_ref, u_hbm, x_hbm, wq_hbm, wk_hbm, wv_hbm, wo_hbm,
            o_hbm,
            raw_q, raw_k, raw_v, u_ref, x_v, wqkv, wo, ob,
            pw, cst, up, yp, dsk, sems, *slots,
            L, D, N, H, Dh, M, SEG):
    sre, sim, zre, zim, tre, tim = (slots[i::6] for i in range(6))
    NC = L // T
    NB = D // 128
    NSEG = L // SEG
    R = M + SEG

    NO = NSEG // PER
    X0 = PER * SEG
    copy = pltpu.make_async_copy
    load_u = copy(u_hbm, u_ref.at[pl.ds(0, L), :], sems.at[0])
    load_w = [copy(w.bitcast(U32), r, sems.at[1 + i])
              for i, (w, r) in enumerate(((wq_hbm, raw_q), (wk_hbm, raw_k), (wv_hbm, raw_v)))]
    load_wo = copy(wo_hbm.bitcast(U32), wo, sems.at[4])
    load_x0 = copy(x_hbm.at[pl.ds(0, X0), :], x_v.at[pl.ds(0, X0), :], sems.at[5])
    load_x1 = copy(x_hbm.at[pl.ds(X0, L - X0), :], x_v.at[pl.ds(X0, L - X0), :], sems.at[6])
    for c in [load_u] + load_w + [load_wo, load_x0]:
        c.start()

    lane = lax.broadcasted_iota(jnp.int32, (T, 128), 1)
    lo64 = lane < 64
    lo32 = lax.broadcasted_iota(jnp.int32, (NC, 128), 1) < 64

    ldt = ldt_ref[...].astype(F32).reshape(1, D)
    dsk[...] = dsk_ref[...].astype(F32).reshape(1, D)
    for b in range(NB):
        rows = slice(b * 128, (b + 1) * 128)
        dt = jnp.exp(ldt[:, rows])
        dt = jnp.broadcast_to(dt, (128, 128)).T
        a = dt * are_ref[rows, :].astype(F32)
        th = dt * aim_ref[rows, :].astype(F32)
        ea = jnp.exp(a)
        w = (ea * jnp.cos(th), ea * jnp.sin(th))
        c = _cmul(cre_ref[rows, :].astype(F32), cim_ref[rows, :].astype(F32),
                  dt * bre_ref[rows, :].astype(F32), dt * bim_ref[rows, :].astype(F32))
        sq = [w]
        for _ in range(6):
            sq.append(_cmul(*sq[-1], *sq[-1]))
        p = [_csqrt(*c)]
        for i in (1, 2, 3):
            p += [_cmul(*x, *sq[i]) for x in p]
        for ri in range(2):
            for j in range(8):
                pw[ri, pl.ds(b * 128 * PP + j * 4, 128, stride=PP), :] = p[j][ri]
            for n, x in enumerate((w, sq[4], sq[6], p[0])):
                cst[2 * n + ri, rows, :] = x[ri]

    flip = jnp.where(lax.broadcasted_iota(jnp.int32, (T, 2 * T), 0)
                     + lax.broadcasted_iota(jnp.int32, (T, 2 * T), 1) == T, 1.0, 0.0).astype(BF16)
    load_u.wait()
    u_ref[L:L + T, :] = jnp.zeros((T, D), BF16)
    u0 = u_ref[0:16, :].astype(F32)[0:1]
    for b in range(NB):
        rows = slice(b * 128, (b + 1) * 128)
        cst[8, rows, :] = jnp.broadcast_to(u0[:, rows], (128, 128)).T

    def u_body(j, carry):
        cs = [j * UC + i for i in range(UC)]
        ns = [_dot(flip, u_ref[pl.ds(pl.multiple_of(c * T, T), 2 * T), :]) for c in cs]
        ns = [_pack(ns[i], ns[i + 1]) for i in range(0, UC, 2)]
        cs = [j * (UC // 2) + i for i in range(UC // 2)]
        stores = []
        for c, n in zip(cs, ns):
            for sb in range(NB // 2):
                xt = jnp.concatenate([n[:, sb * 256:sb * 256 + 128], n[:, sb * 256 + 128:sb * 256 + 256]], axis=0).T
                stores.append((pl.ds(sb * 128 * UP + c, 128, stride=UP), xt))
        if NB % 2:
            for i in range(0, UC // 2, 2):
                n0, n1 = ns[i][:, D - 128:], ns[i + 1][:, D - 128:]
                top = jnp.where(lo64, n0, pltpu.roll(n1, 64, 1))
                bot = jnp.where(lo64, pltpu.roll(n0, 64, 1), n1)
                xt = jnp.concatenate([top, bot], axis=0).T
                for cc in range(2):
                    stores.append((pl.ds((NB // 2) * 128 * UP + cs[i + cc], 64, stride=UP), xt[cc * 64:(cc + 1) * 64]))
        for rows, val in stores:
            up[rows, :] = val
        return carry

    lax.fori_loop(0, NC // UC, u_body, 0)

    r2 = 2 * lax.broadcasted_iota(jnp.int32, (T // 2, 128), 0)
    l2 = lax.broadcasted_iota(jnp.int32, (T // 2, 128), 1)
    hank_ok = (l2 % T) + r2 >= T - 1
    hank_idx = jnp.where(hank_ok, l2 + r2 - (T - 1), l2)
    hank_lo, hank_hi = hank_ok & (l2 < T), hank_ok & (l2 >= T)
    lane8 = lax.broadcasted_iota(jnp.int32, (8, 128), 1)
    not_k = lax.broadcasted_iota(jnp.int32, (8, 128), 0) != 0

    def chans(g):
        ca = (g // 16) * 256 + (g % 16) * 8
        ch = [ca, ca + 128 - 64 * (g // (16 * (NB // 2)))]
        return ch if isinstance(g, int) else [pl.multiple_of(c, 8) for c in ch]

    def lhs(g, p):
        return pltpu.bitcast(up[pl.ds((g * 8 + p) * UP, NC // 2), :], BF16)

    NG = D // 16

    def s4_slot(tau, g0, live):
        def item(lag):
            g, p = divmod(tau - lag, 8)
            return (g, p) if 0 <= g < NG else (None, None)

        stores = []
        g, p = item(T_STATE)
        if g is not None:
            tr, ti = live.pop(("v", g % 3, p))
            x = lhs(g0 + g, p)
            x = jnp.concatenate([jnp.where(lo32, x, 0.0), jnp.where(lo32, 0.0, x)], axis=0)
            live["s", g % 3, p] = _dot(x, pltpu.bitcast(jnp.concatenate([tr, ti], axis=1), BF16))
            stores += [(tre[g % 3], (p,), tr), (tim[g % 3], (p,), ti)]
        g, p = item(T_TAPS)
        if g is not None:
            rows = pl.ds(p * ZP, NC)
            y = (_dot(pltpu.bitcast(zre[g % 3][rows, :], BF16), pltpu.bitcast(tre[g % 3][p], BF16), _NT)
                 - _dot(pltpu.bitcast(zim[g % 3][rows, :], BF16), pltpu.bitcast(tim[g % 3][p], BF16), _NT))
            k2 = jnp.where(lane8 < 64, y[0:8], y[NC:NC + 8])
            k1 = jnp.where(lane8 % T == 0, 0.0, pltpu.roll(k2, 1, 1))
            kq = _pack(k1, k2)
            kq = jnp.broadcast_to(kq[0:1, :], (T // 2, 128))
            live["h", g % 3, p] = jnp.take_along_axis(kq, hank_idx, axis=1)
            first = jnp.where(lane8 < 64, *[jnp.broadcast_to(cst[8, pl.ds(c + p, 1), :], (8, 128)) for c in chans(g0 + g)])
            live["y", g % 3, p] = jnp.concatenate(
                [jnp.where(not_k, k2, k2 * first), jnp.where(lo32[8:], y[8:NC], y[NC + 8:])], axis=0)
        g, p = item(T_INTRA)
        if g is not None:
            hk = live.pop(("h", g % 3, p))
            hk = jnp.concatenate([jnp.where(hank_lo, hk, U32(0)), jnp.where(hank_hi, hk, U32(0))], axis=0)
            live["y", g % 3, p] = live["y", g % 3, p] + _dot(lhs(g0 + g, p), pltpu.bitcast(hk, BF16))
        g, p = item(0)
        if g is not None:
            ch = chans(g0 + g)
            vr, vi = [], []
            for hf in range(2):
                base = pl.ds((ch[hf] + p) * PP, 8, stride=4)
                ev = (pw[0, base, :], pw[1, base, :])
                bc = [jnp.broadcast_to(cst[n, pl.ds(ch[hf] + p, 1), :], (8, 128)) for n in range(4)]
                od = _cmul(*ev, bc[0], bc[1])
                for k in range(T // 16):
                    vr.append(_pack(ev[0], od[0]))
                    vi.append(_pack(ev[1], od[1]))
                    if k + 1 < T // 16:
                        ev = _cmul(*ev, bc[2], bc[3])
                        od = _cmul(*od, bc[2], bc[3])
            live["v", g % 3, p] = (jnp.concatenate(vr, axis=0), jnp.concatenate(vi, axis=0))
        g, p = item(T_SCAN + 1)
        if g is not None:
            for (hf, c), (zr, zi) in live.pop(("z", g % 3, p)).items():
                rows = (pl.ds((hf * NC + c) // 2, 8, stride=ZP), slice(None))
                stores += [(zre[g % 3], rows, zr), (zim[g % 3], rows, zi)]
        g, p = item(T_SCAN)
        if g is not None:
            ch = chans(g0 + g)
            z = {}
            for hf in range(2):
                wtr, wti = [cst[4 + n, pl.ds(ch[hf], 8), :] for n in range(2)]
                if p == 0:
                    live["e", hf] = [cst[6 + n, pl.ds(ch[hf], 8), :] for n in range(2)]
                    live["x", hf] = [x * cst[8, pl.ds(ch[hf], 8), :] for x in live["e", hf]]
                for c in range(p * NC // 8, min((p + 1) * NC // 8, NC - 1)):
                    rows = pl.ds(c * SP, 8, stride=4)
                    xr, xi = sre[g % 3][hf, rows, :], sim[g % 3][hf, rows, :]
                    pr, pi = _cmul(*live["x", hf], wtr, wti)
                    zn = live["x", hf] = [pr + xr, pi + xi]
                    if c % 2:
                        live["e", hf] = zn
                    else:
                        z[hf, c] = [_pack(a, b) for a, b in zip(live.pop(("e", hf)), zn)]
            live["z", g % 3, p] = z
        g, p = item(T_STATE + LMM)
        if g is not None:
            s = live.pop(("s", g % 3, p))
            for hf in range(2):
                rows = (hf, pl.ds(p * 4, NC, stride=SP), slice(None))
                stores += [(sre[g % 3], rows, s[hf * NC:(hf + 1) * NC, 0:128]),
                           (sim[g % 3], rows, s[hf * NC:(hf + 1) * NC, 128:256])]
        g, p = item(T_INTRA + LMM)
        if g is not None:
            gg = g0 + g
            rows = (pl.ds(gg * 8 + p, NC, stride=YP), slice(None))
            stores.append((yp, rows, live.pop(("y", g % 3, p))))
        for ref, idx, val in stores:
            ref[idx] = val

    T0 = 8 * (-(-(T_INTRA + LMM) // 8))
    NJ = (8 * NG - T0) // SB
    live = {}
    for tau in range(T0):
        s4_slot(tau, 0, live)

    def grp_body(j, live):
        live = dict(live)
        for tau in range(T0, T0 + SB):
            s4_slot(tau, (SB // 8) * j, live)
        return live

    live = dict(lax.fori_loop(0, NJ, grp_body, live))
    for tau in range(T0 + SB * NJ, 8 * NG + T_INTRA + LMM):
        s4_slot(tau, 0, live)

    def s4_output(s):
        c, sb = s // 2, s % 2
        rows = pl.ds(pl.multiple_of(c * T, T), T)
        res = []
        xt = yp[pl.ds(c * YP + sb * 128, 128), :].T
        for hf in range(2):
            cols = pl.ds(pl.multiple_of(sb * 256 + hf * 128, 128), 128)
            res.append((rows, cols, xt[hf * T:(hf + 1) * T]))
        xt = yp[pl.ds(c * YP + (NB // 2) * 128 - 64, 128), :].T
        res.append((rows, pl.ds(D - 128, 128), jnp.where(lo64, pltpu.roll(xt[0:T], 64, 1), xt[T:2 * T])))
        return [(r, cl, (y + u_ref[r, cl].astype(F32) * dsk[:, cl]).astype(BF16)) for r, cl, y in res]

    for m, raw in enumerate((raw_q, raw_k, raw_v)):
        load_w[m].wait()

        def w_body(j, carry, m=m, raw=raw):
            src = raw[pl.ds(pl.multiple_of(j * WB * H, WB * H), WB * H), :]
            for r in range(WB):
                for i in range(0, H // 2, 8):
                    ab = [src[r * H + o + i:r * H + o + i + 8] for o in (0, H // 2)]
                    for odd in range(2):
                        rows = pl.ds((m * H + 2 * i + odd) * WP + j * WB + r, 8, stride=2 * WP)
                        wqkv[rows, :] = pltpu.pack_elementwise(
                            [x >> 16 for x in ab] if odd else ab, packed_dtype=jnp.uint16)
            return carry

        lax.fori_loop(0, D // 2 // WB, w_body, 0)
    load_wo.wait()

    load_x0.wait()
    load_x1.start()

    row = lax.broadcasted_iota(jnp.int32, (R, R), 0)
    col = lax.broadcasted_iota(jnp.int32, (R, R), 1)
    scale = Dh ** -0.5

    def flush(stores):
        for r, cl, y in stores:
            ob[r, cl] = y

    def segment(s, mem, pending):
        r0 = pl.multiple_of(s * SEG, SEG)
        hid = jnp.concatenate([mem, x_v[pl.ds(r0, SEG), :].astype(F32)], axis=0)
        mask = (row < M) | (row >= col)
        q, k, v, p, o = {}, {}, {}, {}, {}
        acc, h0, step = None, 0, 0
        while h0 < H:
            if step < H:
                w = jnp.concatenate([wqkv[pl.ds((m * H + step) * WP, D // 2), :] for m in range(3)], axis=1)
                r = _dot(hid, pltpu.bitcast(w, BF16))
                q[step] = r[:, 0:Dh] * scale
                k[step] = r[:, Dh:2 * Dh].astype(BF16)
                v[step] = r[:, 2 * Dh:3 * Dh].astype(BF16)
            h = step - LQK
            if 0 <= h < H:
                sc = jnp.where(mask, _dot(q.pop(h), k.pop(h), _NT), -1e9)
                e = jnp.exp(sc - jnp.max(sc, axis=-1, keepdims=True))
                p[h] = e / jnp.sum(e, axis=-1, keepdims=True)
            h = step - LPV
            if 0 <= h < H:
                o[h] = _dot(p.pop(h), v.pop(h))
            h = h0 + GW - 1
            if h in o and (h <= step - LWO or step >= H):
                oo = jnp.concatenate([o.pop(i) for i in range(h0, h + 1)], axis=1)
                d = _dot(oo, pltpu.bitcast(wo[pl.ds(h0 * Dh // 2, GW * Dh // 2), :], BF16))
                acc = d if acc is None else acc + d
                h0 += GW
            if step == 2:
                flush(pending)
            if step == YSTEP:
                s4_out = s4_output(s)
            if step == YSTEP + 4:
                flush(s4_out)
            step += 1
        return acc[0:M], [(pl.ds(r0, SEG), slice(D, 2 * D), acc[M:R].astype(BF16))]

    def store(j):
        rows = pl.ds(pl.multiple_of(j * X0, X0), X0)
        return copy(ob.at[rows, :], o_hbm.at[rows, :], sems.at[7])

    def outer(j, mem):
        pending = []
        for i in range(PER):
            mem, pending = segment(j * PER + i, mem, pending)
        flush(pending)
        store(j).start()

        @pl.when(j == 0)
        def _():
            load_x1.wait()

        return mem

    lax.fori_loop(0, NO, outer, mem_ref[...].astype(F32))
    copy(ob, o_hbm, sems.at[7]).wait()


@functools.partial(jax.jit, static_argnames=("B_seg_len",))
def pallas_concat_heads__ssm_conv_s4__memory_aug_recurrent_mem_tr__prompt_kernel(
    A_u, A_A_re, A_A_im, A_B_re, A_B_im, A_C_re, A_C_im, A_log_dt, A_Dskip,
    B_x, B_mem0, B_Wq, B_Wk, B_Wv, B_Wo, B_seg_len,
):
    Bsz, L, D = A_u.shape
    N = A_A_re.shape[1]
    _, H, Dh = B_Wq.shape
    M = B_mem0.shape[1]
    SEG = int(B_seg_len)
    assert SEG * 2 == T and D == 640 and Bsz == 1 and B_x.shape == A_u.shape and N == 128 and Dh == 128
    NC = L // T
    NB = D // 128

    vmem = pl.BlockSpec(memory_space=pltpu.VMEM)
    hbm = pl.BlockSpec(memory_space=pl.ANY)
    scratch = [
        pltpu.VMEM((D * H // 2, Dh), U32), pltpu.VMEM((D * H // 2, Dh), U32), pltpu.VMEM((D * H // 2, Dh), U32),
        pltpu.VMEM((L + T, D), BF16),
        pltpu.VMEM((L, D), BF16),
        pltpu.VMEM(((3 * H + 2) * WP, Dh), U32),
        pltpu.VMEM((H * Dh // 2, D), U32),
        pltpu.VMEM((L, 2 * D), BF16),
        pltpu.VMEM((2, (D + 1) * PP, N), F32),
        pltpu.VMEM((9, D, N), F32),
        pltpu.VMEM(((D // 2 + 1) * UP, 128), U32),
        pltpu.VMEM(((NC + 1) * YP, 128), F32),
        pltpu.VMEM((1, D), F32),
        pltpu.SemaphoreType.DMA((8,)),
    ] + 3 * [
        pltpu.VMEM((2, (NC + 1) * SP, N), F32),
        pltpu.VMEM((2, (NC + 1) * SP, N), F32),
        pltpu.VMEM((10 * ZP, N), U32),
        pltpu.VMEM((10 * ZP, N), U32),
        pltpu.VMEM((8, T, N), U32),
        pltpu.VMEM((8, T, N), U32),
    ]
    out = pl.pallas_call(
        functools.partial(_kernel, L=L, D=D, N=N, H=H, Dh=Dh, M=M, SEG=SEG),
        out_shape=jax.ShapeDtypeStruct((L, 2 * D), A_u.dtype),
        in_specs=[vmem] * 9 + [hbm] * 6,
        out_specs=hbm,
        scratch_shapes=scratch,
        compiler_params=pltpu.CompilerParams(vmem_limit_bytes=120 * 1024 * 1024),
        name="s4_rmt",
    )(A_A_re, A_A_im, A_B_re, A_B_im, A_C_re, A_C_im,
      A_log_dt, A_Dskip, B_mem0.reshape(M, D),
      A_u.reshape(L, D), B_x.reshape(L, D), B_Wq.reshape(D * H, Dh), B_Wk.reshape(D * H, Dh),
      B_Wv.reshape(D * H, Dh), B_Wo.reshape(H * Dh, D))
    return out.reshape(Bsz, L, 2 * D)
```

```python
import functools

import jax
import jax.numpy as jnp
from jax import lax
import jax.experimental.pallas as pl
import jax.experimental.pallas.tpu as pltpu

F32 = jnp.float32
BF16 = jnp.bfloat16
U32 = jnp.uint32

LMM, T_STATE, T_SCAN, T_TAPS, T_INTRA = 2, 1, 12, 22, 30
SB = 144
WB = 32
PER = 4
EARLY = 3
UC = 8
YSTEP = 16
T = 64
LQK, LPV, LWO, GW = 2, 6, 20, 2

PP, UP, YP, SP, ZP, WP = 33, 17, 321, 33, 33, 322

_NN = (((1,), (0,)), ((), ()))
_NT = (((1,), (1,)), ((), ()))


def _dot(a, b, dims=_NN):
    return lax.dot_general(a, b, dims, preferred_element_type=F32)


def _pack(a, b):
    return pltpu.pack_elementwise([a, b], packed_dtype=BF16)


def _cmul(ar, ai, br, bi):
    return ar * br - ai * bi, ar * bi + ai * br


def _csqrt(re, im):
    m = jnp.maximum(jnp.abs(re), jnp.abs(im))
    nz = m > 0
    inv = 1.0 / jnp.where(nz, m, 1.0)
    a, b = jnp.where(nz, re * inv, 1.0), im * inv
    r2 = a * a + b * b
    t2 = 0.5 * (r2 * lax.rsqrt(r2) + jnp.abs(a))
    rs = lax.rsqrt(t2)
    big, small = t2 * rs, 0.5 * b * rs
    sm = jnp.sqrt(m)
    return jnp.where(a >= 0, big, small) * sm, jnp.where(a >= 0, small, big) * sm


def _kernel(are_ref, aim_ref, bre_ref, bim_ref, cre_ref, cim_ref, ldt_ref, dsk_ref,
            mem_ref, u_hbm, x_hbm, wq_hbm, wk_hbm, wv_hbm, wo_hbm,
            o_hbm,
            raw_q, raw_k, raw_v, u_ref, x_v, wqkv, wo, ob,
            pw, cst, up, yp, dsk, sems, *slots,
            L, D, N, H, Dh, M, SEG):
    sre, sim, zre, zim, tre, tim = (slots[i::6] for i in range(6))
    NC = L // T
    NB = D // 128
    NSEG = L // SEG
    R = M + SEG

    NO = NSEG // PER
    X0 = PER * SEG
    copy = pltpu.make_async_copy
    load_u = copy(u_hbm, u_ref.at[pl.ds(0, L), :], sems.at[0])
    load_w = [copy(w.bitcast(U32), r, sems.at[1 + i])
              for i, (w, r) in enumerate(((wq_hbm, raw_q), (wk_hbm, raw_k), (wv_hbm, raw_v)))]
    load_wo = copy(wo_hbm.bitcast(U32), wo, sems.at[4])
    load_x0 = copy(x_hbm.at[pl.ds(0, X0), :], x_v.at[pl.ds(0, X0), :], sems.at[5])
    load_x1 = copy(x_hbm.at[pl.ds(X0, L - X0), :], x_v.at[pl.ds(X0, L - X0), :], sems.at[6])
    for c in [load_u] + load_w + [load_wo, load_x0]:
        c.start()

    lane = lax.broadcasted_iota(jnp.int32, (T, 128), 1)
    lo64 = lane < 64
    lo32 = lax.broadcasted_iota(jnp.int32, (NC, 128), 1) < 64

    ldt = ldt_ref[...].astype(F32).reshape(1, D)
    dsk[...] = dsk_ref[...].astype(F32).reshape(1, D)

    def constants(b):
        rows = slice(b * 128, (b + 1) * 128)
        dt = jnp.exp(ldt[:, rows])
        dt = jnp.broadcast_to(dt, (128, 128)).T
        a = dt * are_ref[rows, :].astype(F32)
        th = dt * aim_ref[rows, :].astype(F32)
        ea = jnp.exp(a)
        w = (ea * jnp.cos(th), ea * jnp.sin(th))
        c = _cmul(cre_ref[rows, :].astype(F32), cim_ref[rows, :].astype(F32),
                  dt * bre_ref[rows, :].astype(F32), dt * bim_ref[rows, :].astype(F32))
        sq = [w]
        for _ in range(6):
            sq.append(_cmul(*sq[-1], *sq[-1]))
        p = [_csqrt(*c)]
        for i in (1, 2, 3):
            p += [_cmul(*x, *sq[i]) for x in p]
        for ri in range(2):
            for j in range(8):
                pw[ri, pl.ds(b * 128 * PP + j * 4, 128, stride=PP), :] = p[j][ri]
            for n, x in enumerate((w, sq[4], sq[6], p[0])):
                cst[2 * n + ri, rows, :] = x[ri]

    flip = jnp.where(lax.broadcasted_iota(jnp.int32, (T, 2 * T), 0)
                     + lax.broadcasted_iota(jnp.int32, (T, 2 * T), 1) == T, 1.0, 0.0).astype(BF16)
    for b in range(EARLY):
        constants(b)
    load_u.wait()
    u_ref[L:L + T, :] = jnp.zeros((T, D), BF16)
    u0 = u_ref[0:16, :].astype(F32)[0:1]
    for b in range(NB):
        rows = slice(b * 128, (b + 1) * 128)
        cst[8, rows, :] = jnp.broadcast_to(u0[:, rows], (128, 128)).T

    def u_body(j, carry):
        cs = [j * UC + i for i in range(UC)]
        ns = [_dot(flip, u_ref[pl.ds(c * T, 2 * T), :]) for c in cs]
        ns = [_pack(ns[i], ns[i + 1]) for i in range(0, UC, 2)]
        cs = [j * (UC // 2) + i for i in range(UC // 2)]
        stores = []
        for c, n in zip(cs, ns):
            for sb in range(NB // 2):
                xt = jnp.concatenate([n[:, sb * 256:sb * 256 + 128], n[:, sb * 256 + 128:sb * 256 + 256]], axis=0).T
                stores.append((pl.ds(sb * 128 * UP + c, 128, stride=UP), xt))
        if NB % 2:
            for i in range(0, UC // 2, 2):
                n0, n1 = ns[i][:, D - 128:], ns[i + 1][:, D - 128:]
                top = jnp.where(lo64, n0, pltpu.roll(n1, 64, 1))
                bot = jnp.where(lo64, pltpu.roll(n0, 64, 1), n1)
                xt = jnp.concatenate([top, bot], axis=0).T
                for cc in range(2):
                    stores.append((pl.ds((NB // 2) * 128 * UP + cs[i + cc], 64, stride=UP), xt[cc * 64:(cc + 1) * 64]))
        for rows, val in stores:
            up[rows, :] = val
        return carry

    for j in range(NC // UC):
        u_body(j, 0)
        if EARLY + j < NB:
            constants(EARLY + j)
    for b in range(EARLY + NC // UC, NB):
        constants(b)

    r2 = 2 * lax.broadcasted_iota(jnp.int32, (T // 2, 128), 0)
    l2 = lax.broadcasted_iota(jnp.int32, (T // 2, 128), 1)
    hank_ok = (l2 % T) + r2 >= T - 1
    hank_idx = jnp.where(hank_ok, l2 + r2 - (T - 1), l2)
    hank_lo, hank_hi = hank_ok & (l2 < T), hank_ok & (l2 >= T)
    lane8 = lax.broadcasted_iota(jnp.int32, (8, 128), 1)
    not_k = lax.broadcasted_iota(jnp.int32, (8, 128), 0) != 0

    def chans(g):
        ca = (g // 16) * 256 + (g % 16) * 8
        ch = [ca, ca + 128 - 64 * (g // (16 * (NB // 2)))]
        return ch if isinstance(g, int) else [pl.multiple_of(c, 8) for c in ch]

    def lhs(g, p):
        return pltpu.bitcast(up[pl.ds((g * 8 + p) * UP, NC // 2), :], BF16)

    NG = D // 16

    def s4_slot(tau, g0, live):
        def item(lag):
            g, p = divmod(tau - lag, 8)
            return (g, p) if 0 <= g < NG else (None, None)

        stores = []
        g, p = item(T_STATE)
        if g is not None:
            tr, ti = live.pop(("v", g % 3, p))
            x = lhs(g0 + g, p)
            x = jnp.concatenate([jnp.where(lo32, x, 0.0), jnp.where(lo32, 0.0, x)], axis=0)
            live["s", g % 3, p] = _dot(x, pltpu.bitcast(jnp.concatenate([tr, ti], axis=1), BF16))
            stores += [(tre[g % 3], (p,), tr), (tim[g % 3], (p,), ti)]
        g, p = item(T_TAPS)
        if g is not None:
            rows = pl.ds(p * ZP, NC)
            y = (_dot(pltpu.bitcast(zre[g % 3][rows, :], BF16), pltpu.bitcast(tre[g % 3][p], BF16), _NT)
                 - _dot(pltpu.bitcast(zim[g % 3][rows, :], BF16), pltpu.bitcast(tim[g % 3][p], BF16), _NT))
            k2 = jnp.where(lane8 < 64, y[0:8], y[NC:NC + 8])
            k1 = jnp.where(lane8 % T == 0, 0.0, pltpu.roll(k2, 1, 1))
            kq = _pack(k1, k2)
            kq = jnp.broadcast_to(kq[0:1, :], (T // 2, 128))
            live["h", g % 3, p] = jnp.take_along_axis(kq, hank_idx, axis=1)
            first = jnp.where(lane8 < 64, *[jnp.broadcast_to(cst[8, pl.ds(c + p, 1), :], (8, 128)) for c in chans(g0 + g)])
            live["y", g % 3, p] = jnp.concatenate(
                [jnp.where(not_k, k2, k2 * first), jnp.where(lo32[8:], y[8:NC], y[NC + 8:])], axis=0)
        g, p = item(T_INTRA)
        if g is not None:
            hk = live.pop(("h", g % 3, p))
            hk = jnp.concatenate([jnp.where(hank_lo, hk, U32(0)), jnp.where(hank_hi, hk, U32(0))], axis=0)
            live["y", g % 3, p] = live["y", g % 3, p] + _dot(lhs(g0 + g, p), pltpu.bitcast(hk, BF16))
        g, p = item(0)
        if g is not None:
            ch = chans(g0 + g)
            vr, vi = [], []
            for hf in range(2):
                base = pl.ds((ch[hf] + p) * PP, 8, stride=4)
                ev = (pw[0, base, :], pw[1, base, :])
                bc = [jnp.broadcast_to(cst[n, pl.ds(ch[hf] + p, 1), :], (8, 128)) for n in range(4)]
                od = _cmul(*ev, bc[0], bc[1])
                for k in range(T // 16):
                    vr.append(_pack(ev[0], od[0]))
                    vi.append(_pack(ev[1], od[1]))
                    if k + 1 < T // 16:
                        ev = _cmul(*ev, bc[2], bc[3])
                        od = _cmul(*od, bc[2], bc[3])
            live["v", g % 3, p] = (jnp.concatenate(vr, axis=0), jnp.concatenate(vi, axis=0))
        g, p = item(T_SCAN + 1)
        if g is not None:
            for (hf, c), (zr, zi) in live.pop(("z", g % 3, p)).items():
                rows = (pl.ds((hf * NC + c) // 2, 8, stride=ZP), slice(None))
                stores += [(zre[g % 3], rows, zr), (zim[g % 3], rows, zi)]
        g, p = item(T_SCAN)
        if g is not None:
            ch = chans(g0 + g)
            z = {}
            for hf in range(2):
                wtr, wti = [cst[4 + n, pl.ds(ch[hf], 8), :] for n in range(2)]
                if p == 0:
                    live["e", hf] = [cst[6 + n, pl.ds(ch[hf], 8), :] for n in range(2)]
                    live["x", hf] = [x * cst[8, pl.ds(ch[hf], 8), :] for x in live["e", hf]]
                for c in range(p * NC // 8, min((p + 1) * NC // 8, NC - 1)):
                    rows = pl.ds(c * SP, 8, stride=4)
                    xr, xi = sre[g % 3][hf, rows, :], sim[g % 3][hf, rows, :]
                    pr, pi = _cmul(*live["x", hf], wtr, wti)
                    zn = live["x", hf] = [pr + xr, pi + xi]
                    if c % 2:
                        live["e", hf] = zn
                    else:
                        z[hf, c] = [_pack(a, b) for a, b in zip(live.pop(("e", hf)), zn)]
            live["z", g % 3, p] = z
        g, p = item(T_STATE + LMM)
        if g is not None:
            s = live.pop(("s", g % 3, p))
            for hf in range(2):
                rows = (hf, pl.ds(p * 4, NC, stride=SP), slice(None))
                stores += [(sre[g % 3], rows, s[hf * NC:(hf + 1) * NC, 0:128]),
                           (sim[g % 3], rows, s[hf * NC:(hf + 1) * NC, 128:256])]
        g, p = item(T_INTRA + LMM)
        if g is not None:
            gg = g0 + g
            rows = (pl.ds(gg * 8 + p, NC, stride=YP), slice(None))
            stores.append((yp, rows, live.pop(("y", g % 3, p))))
        for ref, idx, val in stores:
            ref[idx] = val

    T0 = 8 * (-(-(T_INTRA + LMM) // 8))
    NJ = (8 * NG - T0) // SB
    live = {}
    for tau in range(T0):
        s4_slot(tau, 0, live)

    def grp_body(j, live):
        live = dict(live)
        for tau in range(T0, T0 + SB):
            s4_slot(tau, (SB // 8) * j, live)
        return live

    live = dict(lax.fori_loop(0, NJ, grp_body, live))
    for tau in range(T0 + SB * NJ, 8 * NG + T_INTRA + LMM):
        s4_slot(tau, 0, live)

    def s4_output(s):
        c, sb = s // 2, s % 2
        rows = pl.ds(pl.multiple_of(c * T, T), T)
        res = []
        xt = yp[pl.ds(c * YP + sb * 128, 128), :].T
        for hf in range(2):
            cols = pl.ds(pl.multiple_of(sb * 256 + hf * 128, 128), 128)
            res.append((rows, cols, xt[hf * T:(hf + 1) * T]))
        xt = yp[pl.ds(c * YP + (NB // 2) * 128 - 64, 128), :].T
        res.append((rows, pl.ds(D - 128, 128), jnp.where(lo64, pltpu.roll(xt[0:T], 64, 1), xt[T:2 * T])))
        return [(r, cl, (y + u_ref[r, cl].astype(F32) * dsk[:, cl]).astype(BF16)) for r, cl, y in res]

    for m, raw in enumerate((raw_q, raw_k, raw_v)):
        load_w[m].wait()

        def w_body(j, carry, m=m, raw=raw):
            src = raw[pl.ds(pl.multiple_of(j * WB * H, WB * H), WB * H), :]
            for r in range(WB):
                for i in range(0, H // 2, 8):
                    ab = [src[r * H + o + i:r * H + o + i + 8] for o in (0, H // 2)]
                    for odd in range(2):
                        rows = pl.ds((m * H + 2 * i + odd) * WP + j * WB + r, 8, stride=2 * WP)
                        wqkv[rows, :] = pltpu.pack_elementwise(
                            [x >> 16 for x in ab] if odd else ab, packed_dtype=jnp.uint16)
            return carry

        lax.fori_loop(0, D // 2 // WB, w_body, 0)
    load_wo.wait()

    load_x0.wait()
    load_x1.start()

    row = lax.broadcasted_iota(jnp.int32, (R, R), 0)
    col = lax.broadcasted_iota(jnp.int32, (R, R), 1)
    scale = Dh ** -0.5

    def flush(stores):
        for r, cl, y in stores:
            ob[r, cl] = y

    def segment(s, mem, pending):
        r0 = pl.multiple_of(s * SEG, SEG)
        hid = jnp.concatenate([mem, x_v[pl.ds(r0, SEG), :].astype(F32)], axis=0)
        mask = (row < M) | (row >= col)
        q, k, v, p, o = {}, {}, {}, {}, {}
        acc, h0, step = None, 0, 0
        while h0 < H:
            if step < H:
                w = jnp.concatenate([wqkv[pl.ds((m * H + step) * WP, D // 2), :] for m in range(3)], axis=1)
                r = _dot(hid, pltpu.bitcast(w, BF16))
                q[step] = r[:, 0:Dh] * scale
                k[step] = r[:, Dh:2 * Dh].astype(BF16)
                v[step] = r[:, 2 * Dh:3 * Dh].astype(BF16)
            h = step - LQK
            if 0 <= h < H:
                sc = jnp.where(mask, _dot(q.pop(h), k.pop(h), _NT), -1e9)
                e = jnp.exp(sc - jnp.max(sc, axis=-1, keepdims=True))
                p[h] = e / jnp.sum(e, axis=-1, keepdims=True)
            h = step - LPV
            if 0 <= h < H:
                o[h] = _dot(p.pop(h), v.pop(h))
            h = h0 + GW - 1
            if h in o and (h <= step - LWO or step >= H):
                oo = jnp.concatenate([o.pop(i) for i in range(h0, h + 1)], axis=1)
                d = _dot(oo, pltpu.bitcast(wo[pl.ds(h0 * Dh // 2, GW * Dh // 2), :], BF16))
                acc = d if acc is None else acc + d
                h0 += GW
            if step == 2:
                flush(pending)
            if step == YSTEP:
                s4_out = s4_output(s)
            if step == YSTEP + 4:
                flush(s4_out)
            step += 1
        return acc[0:M], [(pl.ds(r0, SEG), slice(D, 2 * D), acc[M:R].astype(BF16))]

    def store(j):
        rows = pl.ds(pl.multiple_of(j * X0, X0), X0)
        return copy(ob.at[rows, :], o_hbm.at[rows, :], sems.at[7])

    def outer(j, mem):
        pending = []
        for i in range(PER):
            mem, pending = segment(j * PER + i, mem, pending)
        flush(pending)
        store(j).start()

        @pl.when(j == 0)
        def _():
            load_x1.wait()

        return mem

    lax.fori_loop(0, NO, outer, mem_ref[...].astype(F32))
    copy(ob, o_hbm, sems.at[7]).wait()


@functools.partial(jax.jit, static_argnames=("B_seg_len",))
def pallas_concat_heads__ssm_conv_s4__memory_aug_recurrent_mem_tr__prompt_kernel(
    A_u, A_A_re, A_A_im, A_B_re, A_B_im, A_C_re, A_C_im, A_log_dt, A_Dskip,
    B_x, B_mem0, B_Wq, B_Wk, B_Wv, B_Wo, B_seg_len,
):
    Bsz, L, D = A_u.shape
    N = A_A_re.shape[1]
    _, H, Dh = B_Wq.shape
    M = B_mem0.shape[1]
    SEG = int(B_seg_len)
    assert SEG * 2 == T and D == 640 and Bsz == 1 and B_x.shape == A_u.shape and N == 128 and Dh == 128
    NC = L // T
    NB = D // 128

    vmem = pl.BlockSpec(memory_space=pltpu.VMEM)
    hbm = pl.BlockSpec(memory_space=pl.ANY)
    scratch = [
        pltpu.VMEM((D * H // 2, Dh), U32), pltpu.VMEM((D * H // 2, Dh), U32), pltpu.VMEM((D * H // 2, Dh), U32),
        pltpu.VMEM((L + T, D), BF16),
        pltpu.VMEM((L, D), BF16),
        pltpu.VMEM(((3 * H + 2) * WP, Dh), U32),
        pltpu.VMEM((H * Dh // 2, D), U32),
        pltpu.VMEM((L, 2 * D), BF16),
        pltpu.VMEM((2, (D + 1) * PP, N), F32),
        pltpu.VMEM((9, D, N), F32),
        pltpu.VMEM(((D // 2 + 1) * UP, 128), U32),
        pltpu.VMEM(((NC + 1) * YP, 128), F32),
        pltpu.VMEM((1, D), F32),
        pltpu.SemaphoreType.DMA((8,)),
    ] + 3 * [
        pltpu.VMEM((2, (NC + 1) * SP, N), F32),
        pltpu.VMEM((2, (NC + 1) * SP, N), F32),
        pltpu.VMEM((10 * ZP, N), U32),
        pltpu.VMEM((10 * ZP, N), U32),
        pltpu.VMEM((8, T, N), U32),
        pltpu.VMEM((8, T, N), U32),
    ]
    out = pl.pallas_call(
        functools.partial(_kernel, L=L, D=D, N=N, H=H, Dh=Dh, M=M, SEG=SEG),
        out_shape=jax.ShapeDtypeStruct((L, 2 * D), A_u.dtype),
        in_specs=[vmem] * 9 + [hbm] * 6,
        out_specs=hbm,
        scratch_shapes=scratch,
        compiler_params=pltpu.CompilerParams(vmem_limit_bytes=120 * 1024 * 1024),
        name="s4_rmt",
    )(A_A_re, A_A_im, A_B_re, A_B_im, A_C_re, A_C_im,
      A_log_dt, A_Dskip, B_mem0.reshape(M, D),
      A_u.reshape(L, D), B_x.reshape(L, D), B_Wq.reshape(D * H, Dh), B_Wk.reshape(D * H, Dh),
      B_Wv.reshape(D * H, Dh), B_Wo.reshape(H * Dh, D))
    return out.reshape(Bsz, L, 2 * D)
```

```python
import functools

import numpy as np
import jax
import jax.numpy as jnp
from jax import lax
import jax.experimental.pallas as pl
import jax.experimental.pallas.tpu as pltpu

F32 = jnp.float32
BF16 = jnp.bfloat16
U32 = jnp.uint32

LMM, T_STATE, T_SCAN, T_TAPS, T_INTRA = 2, 1, 12, 22, 30
SB = 144
WB = 32
PER = 4
EARLY = 3
UC = 8
YSTEP = 16
T = 64
LQK, LPV, LWO, GW = 2, 6, 20, 2

PP, UP, YP, SP, ZP, WP = 33, 17, 321, 33, 33, 322

_NN = (((1,), (0,)), ((), ()))
_NT = (((1,), (1,)), ((), ()))


def _dot(a, b, dims=_NN):
    return lax.dot_general(a, b, dims, preferred_element_type=F32)


def _pack(a, b):
    return pltpu.pack_elementwise([a, b], packed_dtype=BF16)


def _cmul(ar, ai, br, bi):
    return ar * br - ai * bi, ar * bi + ai * br


def _csqrt(re, im):
    m = jnp.maximum(jnp.abs(re), jnp.abs(im))
    nz = m > 0
    inv = 1.0 / jnp.where(nz, m, 1.0)
    a, b = jnp.where(nz, re * inv, 1.0), im * inv
    r2 = a * a + b * b
    t2 = 0.5 * (r2 * lax.rsqrt(r2) + jnp.abs(a))
    rs = lax.rsqrt(t2)
    big, small = t2 * rs, 0.5 * b * rs
    sm = jnp.sqrt(m)
    return jnp.where(a >= 0, big, small) * sm, jnp.where(a >= 0, small, big) * sm


def _kernel(are_ref, aim_ref, bre_ref, bim_ref, cre_ref, cim_ref, ldt_ref, dsk_ref,
            mem_ref, u_hbm, x_hbm, wq_hbm, wk_hbm, wv_hbm, wo_hbm,
            o_hbm,
            raw_q, raw_k, raw_v, u_ref, x_v, wqkv, wo, ob,
            pw, cst, up, yp, dsk, sems, *slots,
            L, D, N, H, Dh, M, SEG):
    sre, sim, zre, zim, tre, tim = (slots[i::6] for i in range(6))
    NC = L // T
    NB = D // 128
    NSEG = L // SEG
    R = M + SEG

    NO = NSEG // PER
    X0 = PER * SEG
    copy = pltpu.make_async_copy
    load_u = copy(u_hbm, u_ref.at[pl.ds(0, L), :], sems.at[0])
    load_w = [copy(w.bitcast(U32), r, sems.at[1 + i])
              for i, (w, r) in enumerate(((wq_hbm, raw_q), (wk_hbm, raw_k), (wv_hbm, raw_v)))]
    load_wo = copy(wo_hbm.bitcast(U32), wo, sems.at[4])
    load_x0 = copy(x_hbm.at[pl.ds(0, X0), :], x_v.at[pl.ds(0, X0), :], sems.at[5])
    load_x1 = copy(x_hbm.at[pl.ds(X0, L - X0), :], x_v.at[pl.ds(X0, L - X0), :], sems.at[6])
    for c in [load_u] + load_w + [load_wo, load_x0]:
        c.start()

    lane = lax.broadcasted_iota(jnp.int32, (T, 128), 1)
    lo64 = lane < 64
    lo32 = lax.broadcasted_iota(jnp.int32, (NC, 128), 1) < 64

    ldt = ldt_ref[...].astype(F32).reshape(1, D)
    dsk[...] = dsk_ref[...].astype(F32).reshape(1, D)

    def constants(b):
        rows = slice(b * 128, (b + 1) * 128)
        dt = jnp.exp(ldt[:, rows])
        dt = jnp.broadcast_to(dt, (128, 128)).T
        a = dt * are_ref[rows, :].astype(F32)
        th = dt * aim_ref[rows, :].astype(F32)
        ea = jnp.exp(a)
        w = (ea * jnp.cos(th), ea * jnp.sin(th))
        c = _cmul(cre_ref[rows, :].astype(F32), cim_ref[rows, :].astype(F32),
                  dt * bre_ref[rows, :].astype(F32), dt * bim_ref[rows, :].astype(F32))
        sq = [w]
        for _ in range(6):
            sq.append(_cmul(*sq[-1], *sq[-1]))
        p = [_csqrt(*c)]
        for i in (1, 2, 3):
            p += [_cmul(*x, *sq[i]) for x in p]
        for ri in range(2):
            for j in range(8):
                pw[ri, pl.ds(b * 128 * PP + j * 4, 128, stride=PP), :] = p[j][ri]
            for n, x in enumerate((w, sq[4], sq[6], p[0])):
                cst[2 * n + ri, rows, :] = x[ri]

    flip = jnp.where(lax.broadcasted_iota(jnp.int32, (T, 2 * T), 0)
                     + lax.broadcasted_iota(jnp.int32, (T, 2 * T), 1) == T, 1.0, 0.0).astype(BF16)
    for b in range(EARLY):
        constants(b)
    load_u.wait()
    u_ref[L:L + T, :] = jnp.zeros((T, D), BF16)
    u0 = u_ref[0:16, :].astype(F32)[0:1]
    for b in range(NB):
        rows = slice(b * 128, (b + 1) * 128)
        cst[8, rows, :] = jnp.broadcast_to(u0[:, rows], (128, 128)).T

    def relayout_input(j):
        cs = [j * UC + i for i in range(UC)]
        ns = [_dot(flip, u_ref[pl.ds(c * T, 2 * T), :]) for c in cs]
        ns = [_pack(ns[i], ns[i + 1]) for i in range(0, UC, 2)]
        cs = [j * (UC // 2) + i for i in range(UC // 2)]
        stores = []
        for c, n in zip(cs, ns):
            for sb in range(NB // 2):
                xt = jnp.concatenate([n[:, sb * 256:sb * 256 + 128], n[:, sb * 256 + 128:sb * 256 + 256]], axis=0).T
                stores.append((pl.ds(sb * 128 * UP + c, 128, stride=UP), xt))
        if NB % 2:
            for i in range(0, UC // 2, 2):
                n0, n1 = ns[i][:, D - 128:], ns[i + 1][:, D - 128:]
                top = jnp.where(lo64, n0, pltpu.roll(n1, 64, 1))
                bot = jnp.where(lo64, pltpu.roll(n0, 64, 1), n1)
                xt = jnp.concatenate([top, bot], axis=0).T
                for cc in range(2):
                    stores.append((pl.ds((NB // 2) * 128 * UP + cs[i + cc], 64, stride=UP), xt[cc * 64:(cc + 1) * 64]))
        for rows, val in stores:
            up[rows, :] = val

    for j in range(NC // UC):
        relayout_input(j)
        if EARLY + j < NB:
            constants(EARLY + j)
    for b in range(EARLY + NC // UC, NB):
        constants(b)

    r2 = 2 * lax.broadcasted_iota(jnp.int32, (T // 2, 128), 0)
    l2 = lax.broadcasted_iota(jnp.int32, (T // 2, 128), 1)
    hank_ok = (l2 % T) + r2 >= T - 1
    hank_idx = jnp.where(hank_ok, l2 + r2 - (T - 1), l2)
    hank_lo, hank_hi = hank_ok & (l2 < T), hank_ok & (l2 >= T)
    lane8 = lax.broadcasted_iota(jnp.int32, (8, 128), 1)
    not_k = lax.broadcasted_iota(jnp.int32, (8, 128), 0) != 0

    def chans(g):
        ca = (g // 16) * 256 + (g % 16) * 8
        ch = [ca, ca + 128 - 64 * (g // (16 * (NB // 2)))]
        return ch if isinstance(g, int) else [pl.multiple_of(c, 8) for c in ch]

    def lhs(g, p):
        return pltpu.bitcast(up[pl.ds((g * 8 + p) * UP, NC // 2), :], BF16)

    NG = D // 16

    def s4_slot(tau, g0, live):
        def item(lag):
            g, p = divmod(tau - lag, 8)
            return (g, p) if 0 <= g < NG else (None, None)

        stores = []
        g, p = item(T_STATE)
        if g is not None:
            tr, ti = live.pop(("v", g % 3, p))
            x = lhs(g0 + g, p)
            x = jnp.concatenate([jnp.where(lo32, x, 0.0), jnp.where(lo32, 0.0, x)], axis=0)
            live["s", g % 3, p] = _dot(x, pltpu.bitcast(jnp.concatenate([tr, ti], axis=1), BF16))
            stores += [(tre[g % 3], (p,), tr), (tim[g % 3], (p,), ti)]
        g, p = item(T_TAPS)
        if g is not None:
            rows = pl.ds(p * ZP, NC)
            y = (_dot(pltpu.bitcast(zre[g % 3][rows, :], BF16), pltpu.bitcast(tre[g % 3][p], BF16), _NT)
                 - _dot(pltpu.bitcast(zim[g % 3][rows, :], BF16), pltpu.bitcast(tim[g % 3][p], BF16), _NT))
            k2 = jnp.where(lane8 < 64, y[0:8], y[NC:NC + 8])
            k1 = jnp.where(lane8 % T == 0, 0.0, pltpu.roll(k2, 1, 1))
            kq = _pack(k1, k2)
            kq = jnp.broadcast_to(kq[0:1, :], (T // 2, 128))
            live["h", g % 3, p] = jnp.take_along_axis(kq, hank_idx, axis=1)
            first = jnp.where(lane8 < 64, *[jnp.broadcast_to(cst[8, pl.ds(c + p, 1), :], (8, 128)) for c in chans(g0 + g)])
            live["y", g % 3, p] = jnp.concatenate(
                [jnp.where(not_k, k2, k2 * first), jnp.where(lo32[8:], y[8:NC], y[NC + 8:])], axis=0)
        g, p = item(T_INTRA)
        if g is not None:
            hk = live.pop(("h", g % 3, p))
            hk = jnp.concatenate([jnp.where(hank_lo, hk, np.uint32(0)), jnp.where(hank_hi, hk, np.uint32(0))], axis=0)
            live["y", g % 3, p] = live["y", g % 3, p] + _dot(lhs(g0 + g, p), pltpu.bitcast(hk, BF16))
        g, p = item(0)
        if g is not None:
            ch = chans(g0 + g)
            vr, vi = [], []
            for hf in range(2):
                base = pl.ds((ch[hf] + p) * PP, 8, stride=4)
                ev = (pw[0, base, :], pw[1, base, :])
                bc = [jnp.broadcast_to(cst[n, pl.ds(ch[hf] + p, 1), :], (8, 128)) for n in range(4)]
                od = _cmul(*ev, bc[0], bc[1])
                for k in range(T // 16):
                    vr.append(_pack(ev[0], od[0]))
                    vi.append(_pack(ev[1], od[1]))
                    if k + 1 < T // 16:
                        ev = _cmul(*ev, bc[2], bc[3])
                        od = _cmul(*od, bc[2], bc[3])
            live["v", g % 3, p] = (jnp.concatenate(vr, axis=0), jnp.concatenate(vi, axis=0))
        g, p = item(T_SCAN + 1)
        if g is not None:
            for (hf, c), (zr, zi) in live.pop(("z", g % 3, p)).items():
                rows = (pl.ds((hf * NC + c) // 2, 8, stride=ZP), slice(None))
                stores += [(zre[g % 3], rows, zr), (zim[g % 3], rows, zi)]
        g, p = item(T_SCAN)
        if g is not None:
            ch = chans(g0 + g)
            z = {}
            for hf in range(2):
                wtr, wti = [cst[4 + n, pl.ds(ch[hf], 8), :] for n in range(2)]
                if p == 0:
                    live["e", hf] = [cst[6 + n, pl.ds(ch[hf], 8), :] for n in range(2)]
                    live["x", hf] = [x * cst[8, pl.ds(ch[hf], 8), :] for x in live["e", hf]]
                for c in range(p * NC // 8, min((p + 1) * NC // 8, NC - 1)):
                    rows = pl.ds(c * SP, 8, stride=4)
                    xr, xi = sre[g % 3][hf, rows, :], sim[g % 3][hf, rows, :]
                    pr, pi = _cmul(*live["x", hf], wtr, wti)
                    zn = live["x", hf] = [pr + xr, pi + xi]
                    if c % 2:
                        live["e", hf] = zn
                    else:
                        z[hf, c] = [_pack(a, b) for a, b in zip(live.pop(("e", hf)), zn)]
            live["z", g % 3, p] = z
        g, p = item(T_STATE + LMM)
        if g is not None:
            s = live.pop(("s", g % 3, p))
            for hf in range(2):
                rows = (hf, pl.ds(p * 4, NC, stride=SP), slice(None))
                stores += [(sre[g % 3], rows, s[hf * NC:(hf + 1) * NC, 0:128]),
                           (sim[g % 3], rows, s[hf * NC:(hf + 1) * NC, 128:256])]
        g, p = item(T_INTRA + LMM)
        if g is not None:
            gg = g0 + g
            rows = (pl.ds(gg * 8 + p, NC, stride=YP), slice(None))
            stores.append((yp, rows, live.pop(("y", g % 3, p))))
        for ref, idx, val in stores:
            ref[idx] = val

    T0 = 8 * (-(-(T_INTRA + LMM) // 8))
    NJ = (8 * NG - T0) // SB
    live = {}
    for tau in range(T0):
        s4_slot(tau, 0, live)

    def grp_body(j, live):
        live = dict(live)
        for tau in range(T0, T0 + SB):
            s4_slot(tau, (SB // 8) * j, live)
        return live

    live = dict(lax.fori_loop(0, NJ, grp_body, live))
    for tau in range(T0 + SB * NJ, 8 * NG + T_INTRA + LMM):
        s4_slot(tau, 0, live)

    def s4_output(s):
        c, sb = s // 2, s % 2
        rows = pl.ds(pl.multiple_of(c * T, T), T)
        res = []
        xt = yp[pl.ds(c * YP + sb * 128, 128), :].T
        for hf in range(2):
            cols = pl.ds(pl.multiple_of(sb * 256 + hf * 128, 128), 128)
            res.append((rows, cols, xt[hf * T:(hf + 1) * T]))
        xt = yp[pl.ds(c * YP + (NB // 2) * 128 - 64, 128), :].T
        res.append((rows, pl.ds(D - 128, 128), jnp.where(lo64, pltpu.roll(xt[0:T], 64, 1), xt[T:2 * T])))
        return [(r, cl, (y + u_ref[r, cl].astype(F32) * dsk[:, cl]).astype(BF16)) for r, cl, y in res]

    for m, raw in enumerate((raw_q, raw_k, raw_v)):
        load_w[m].wait()

        def w_body(j, carry, m=m, raw=raw):
            src = raw[pl.ds(pl.multiple_of(j * WB * H, WB * H), WB * H), :]
            for r in range(WB):
                for i in range(0, H // 2, 8):
                    ab = [src[r * H + o + i:r * H + o + i + 8] for o in (0, H // 2)]
                    for odd in range(2):
                        rows = pl.ds((m * H + 2 * i + odd) * WP + j * WB + r, 8, stride=2 * WP)
                        wqkv[rows, :] = pltpu.pack_elementwise(
                            [x >> 16 for x in ab] if odd else ab, packed_dtype=jnp.uint16)
            return carry

        lax.fori_loop(0, D // 2 // WB, w_body, 0)
    load_wo.wait()

    load_x0.wait()
    load_x1.start()

    row = lax.broadcasted_iota(jnp.int32, (R, R), 0)
    col = lax.broadcasted_iota(jnp.int32, (R, R), 1)
    scale = Dh ** -0.5

    def flush(stores):
        for r, cl, y in stores:
            ob[r, cl] = y

    def segment(s, mem, pending):
        r0 = pl.multiple_of(s * SEG, SEG)
        hid = jnp.concatenate([mem, x_v[pl.ds(r0, SEG), :].astype(F32)], axis=0)
        mask = (row < M) | (row >= col)
        q, k, v, p, o = {}, {}, {}, {}, {}
        acc, h0, step = None, 0, 0
        while h0 < H:
            if step < H:
                w = jnp.concatenate([wqkv[pl.ds((m * H + step) * WP, D // 2), :] for m in range(3)], axis=1)
                r = _dot(hid, pltpu.bitcast(w, BF16))
                q[step] = r[:, 0:Dh] * scale
                k[step] = r[:, Dh:2 * Dh].astype(BF16)
                v[step] = r[:, 2 * Dh:3 * Dh].astype(BF16)
            h = step - LQK
            if 0 <= h < H:
                sc = jnp.where(mask, _dot(q.pop(h), k.pop(h), _NT), -1e9)
                e = jnp.exp(sc - jnp.max(sc, axis=-1, keepdims=True))
                p[h] = e / jnp.sum(e, axis=-1, keepdims=True)
            h = step - LPV
            if 0 <= h < H:
                o[h] = _dot(p.pop(h), v.pop(h))
            h = h0 + GW - 1
            if h in o and (h <= step - LWO or step >= H):
                oo = jnp.concatenate([o.pop(i) for i in range(h0, h + 1)], axis=1)
                d = _dot(oo, pltpu.bitcast(wo[pl.ds(h0 * Dh // 2, GW * Dh // 2), :], BF16))
                acc = d if acc is None else acc + d
                h0 += GW
            if step == 2:
                flush(pending)
            if step == YSTEP:
                s4_out = s4_output(s)
            if step == YSTEP + 4:
                flush(s4_out)
            step += 1
        return acc[0:M], [(pl.ds(r0, SEG), slice(D, 2 * D), acc[M:R].astype(BF16))]

    def store(j):
        rows = pl.ds(pl.multiple_of(j * X0, X0), X0)
        return copy(ob.at[rows, :], o_hbm.at[rows, :], sems.at[7])

    def outer(j, mem):
        pending = []
        for i in range(PER):
            mem, pending = segment(j * PER + i, mem, pending)
        flush(pending)
        store(j).start()

        @pl.when(j == 0)
        def _():
            load_x1.wait()

        return mem

    lax.fori_loop(0, NO, outer, mem_ref[...].astype(F32))
    copy(ob, o_hbm, sems.at[7]).wait()


@functools.partial(jax.jit, static_argnames=("B_seg_len",))
def pallas_concat_heads__ssm_conv_s4__memory_aug_recurrent_mem_tr__prompt_kernel(
    A_u, A_A_re, A_A_im, A_B_re, A_B_im, A_C_re, A_C_im, A_log_dt, A_Dskip,
    B_x, B_mem0, B_Wq, B_Wk, B_Wv, B_Wo, B_seg_len,
):
    Bsz, L, D = A_u.shape
    N = A_A_re.shape[1]
    _, H, Dh = B_Wq.shape
    M = B_mem0.shape[1]
    SEG = int(B_seg_len)
    assert SEG * 2 == T and D == 640 and Bsz == 1 and B_x.shape == A_u.shape and N == 128 and Dh == 128
    NC = L // T
    NB = D // 128

    vmem = pl.BlockSpec(memory_space=pltpu.VMEM)
    hbm = pl.BlockSpec(memory_space=pl.ANY)
    scratch = [
        pltpu.VMEM((D * H // 2, Dh), U32), pltpu.VMEM((D * H // 2, Dh), U32), pltpu.VMEM((D * H // 2, Dh), U32),
        pltpu.VMEM((L + T, D), BF16),
        pltpu.VMEM((L, D), BF16),
        pltpu.VMEM(((3 * H + 2) * WP, Dh), U32),
        pltpu.VMEM((H * Dh // 2, D), U32),
        pltpu.VMEM((L, 2 * D), BF16),
        pltpu.VMEM((2, (D + 1) * PP, N), F32),
        pltpu.VMEM((9, D, N), F32),
        pltpu.VMEM(((D // 2 + 1) * UP, 128), U32),
        pltpu.VMEM(((NC + 1) * YP, 128), F32),
        pltpu.VMEM((1, D), F32),
        pltpu.SemaphoreType.DMA((8,)),
    ] + 3 * [
        pltpu.VMEM((2, (NC + 1) * SP, N), F32),
        pltpu.VMEM((2, (NC + 1) * SP, N), F32),
        pltpu.VMEM((10 * ZP, N), U32),
        pltpu.VMEM((10 * ZP, N), U32),
        pltpu.VMEM((8, T, N), U32),
        pltpu.VMEM((8, T, N), U32),
    ]
    out = pl.pallas_call(
        functools.partial(_kernel, L=L, D=D, N=N, H=H, Dh=Dh, M=M, SEG=SEG),
        out_shape=jax.ShapeDtypeStruct((L, 2 * D), A_u.dtype),
        in_specs=[vmem] * 9 + [hbm] * 6,
        out_specs=hbm,
        scratch_shapes=scratch,
        compiler_params=pltpu.CompilerParams(vmem_limit_bytes=120 * 1024 * 1024),
        name="s4_rmt",
    )(A_A_re, A_A_im, A_B_re, A_B_im, A_C_re, A_C_im,
      A_log_dt, A_Dskip, B_mem0.reshape(M, D),
      A_u.reshape(L, D), B_x.reshape(L, D), B_Wq.reshape(D * H, Dh), B_Wk.reshape(D * H, Dh),
      B_Wv.reshape(D * H, Dh), B_Wo.reshape(H * Dh, D))
    return out.reshape(Bsz, L, 2 * D)
```
